```python
import jax
import jax.numpy as jnp

def _softmax(x, axis=-1):
    return jax.nn.softmax(x, axis=axis)
def _gelu(x):
    return jax.nn.gelu(x, approximate=True)
def _silu(x):
    return jax.nn.silu(x)
def _sigmoid(x):
    return jax.nn.sigmoid(x)
def _layernorm(x, axis=-1, eps=1e-5):
    m = jnp.mean(x, axis=axis, keepdims=True)
    v = jnp.var(x, axis=axis, keepdims=True)
    return (x - m) / jnp.sqrt(v + eps)
def _scatter_add(tgt, idx, src, axis=0):
    return tgt.at[idx].add(src)
def _segment_sum(src, seg, n):
    return jax.ops.segment_sum(src, seg, n)
class _Rng:
    def __init__(self, key):
        self._k = key
    def _next(self):
        self._k, sub = jax.random.split(self._k)
        return sub
    def normal(self, shape):
        return jax.random.normal(self._next(), shape, dtype=jnp.bfloat16)
    def randint(self, lo, hi, shape):
        return jax.random.randint(self._next(), shape, lo, hi, dtype=jnp.int32)
    def uniform(self, shape, lo=0.0, hi=1.0):
        return jax.random.uniform(self._next(), shape, jnp.bfloat16, lo, hi)
    def permutation(self, n):
        return jax.random.permutation(self._next(), n)


kernel_name = 'gated_mix__sliding_block_cached__dense_activation_gelu__decode'

def setup_inputs():
    _rng = _Rng(jax.random.key(int.from_bytes(__import__("os").urandom(4), "little")))
    _w = (lambda a: (lambda t: t.astype(jnp.bfloat16) if jnp.issubdtype(t.dtype, jnp.floating) else t)(jnp.asarray(a)))
    def _A_setup():
        B, Sq, D = 1, 1, 640
        Hq, Hkv, Sk, Dh = 32, 32, 32768, 192
        assert Hq % Hkv == 0, (Hq, Hkv)
        return {
            "x": _w((lambda *s: _rng.normal(s) * 0.05)(B, Sq, D)),
            "k_cache": _w((lambda *s: _rng.normal(s) * 0.05)(B, Hkv, Sk, Dh)),
            "v_cache": _w((lambda *s: _rng.normal(s) * 0.05)(B, Hkv, Sk, Dh)),
            "wq": _w((lambda *s: _rng.normal(s) * 0.05)(D, Hq * Dh) * (D ** -0.5)),
            "wo": _w((lambda *s: _rng.normal(s) * 0.05)(Hq * Dh, D) * ((Hq * Dh) ** -0.5)),
        }
    _A_in = _A_setup()

    def _B_setup():
        B, S, D, F = 1, 1, 640, 1536
        return {
            "x": _w((lambda *s: _rng.normal(s) * 0.05)(B, S, D)),
            "w1": _w((lambda *s: _rng.normal(s) * 0.05)(D, F) * (D ** -0.5)),
            "b1": _w((lambda *s: _rng.normal(s) * 0.05)(F) * 0.01),
            "w2": _w((lambda *s: _rng.normal(s) * 0.05)(F, D) * (F ** -0.5)),
            "b2": _w((lambda *s: _rng.normal(s) * 0.05)(D) * 0.01),
        }
    _B_in = _B_setup()

    return {
        "A_x": _A_in["x"],
        "A_k_cache": _A_in["k_cache"],
        "A_v_cache": _A_in["v_cache"],
        "A_wq": _A_in["wq"],
        "A_wo": _A_in["wo"],
        "B_x": _B_in["x"],
        "B_w1": _B_in["w1"],
        "B_b1": _B_in["b1"],
        "B_w2": _B_in["w2"],
        "B_b2": _B_in["b2"],
        "gate_w": _w((lambda *s: _rng.normal(s) * 0.05)(640)),
    }

def reference(A_x, A_k_cache, A_v_cache, A_wq, A_wo, B_x, B_w1, B_b1, B_w2, B_b2, gate_w):
    def _A_ref(x, k_cache, v_cache, wq, wo):
        B, Sq, D = x.shape
        Hq, Dh = 32, 192
        Hkv, Sk = k_cache.shape[1], k_cache.shape[2]
        W = min(4096, max(256, Sk // 4))
        rep = Hq // Hkv
        q = (lambda x, *d: x.transpose(*d))((x @ wq).reshape(B, Sq, Hq, Dh), 0, 2, 1, 3)
        k = jnp.repeat(k_cache[:, :, Sk - W:, :], rep, axis=1)
        v = jnp.repeat(v_cache[:, :, Sk - W:, :], rep, axis=1)
        scores = jnp.einsum("bhqd,bhkd->bhqk", q, k) * (Dh ** -0.5)
        p = _softmax(scores, axis=-1)
        o = jnp.einsum("bhqk,bhkd->bhqd", p, v)
        return (lambda x, *d: x.transpose(*d))(o, 0, 2, 1, 3).reshape(B, Sq, Hq * Dh) @ wo

    def _B_ref(x, w1, b1, w2, b2):
        h = jnp.einsum("bsd,df->bsf", x, w1) + b1
        h = _gelu(h)
        return jnp.einsum("bsf,fd->bsd", h, w2) + b2

    x = A_x
    g = _sigmoid((x * gate_w).sum(-1, keepdims=True))
    a = _A_ref(x, A_k_cache, A_v_cache, A_wq, A_wo)
    b = _B_ref(x, B_w1, B_b1, B_w2, B_b2)
    return g * a + (1 - g) * b
```

```python
import jax
import jax.numpy as jnp
import jax.experimental.pallas as pl
import jax.experimental.pallas.tpu as pltpu

_F32 = jnp.float32
_BF16 = jnp.bfloat16
_LANES = 128

_HQ = 32
_DH = 192


def _interleave(a, b):
    out = []
    for i in range(max(len(a), len(b))):
        if i < len(a):
            out.append(a[i])
        if i < len(b):
            out.append(b[i])
    return out


def _start_all(descs):
    for i, d in enumerate(descs):
        d.start(priority=i % 2)


def _make_kernel(D, F, Sk, W):
    scale = _DH ** -0.5
    n_pairs = _HQ // 2
    pair_w = 2 * _DH
    n_kc = W // _LANES
    col0 = Sk - W
    wq_rows = 160
    w2_blocks = F // _DH

    def kernel(x_hbm, k_hbm, v_hbm, wq_hbm, wo_hbm, w1_hbm, b1_hbm, w2_hbm, b2_hbm, gw_hbm,
               o_ref,
               kbuf, vbuf, wqbuf, wobuf, w1buf, w2buf, xbuf, b1buf, b2buf, gwbuf,
               sem_k, sem_v, sem_wq, sem_wo, sem_w1, sem_w2, sem_s):

        def kv_descs(h, slot):
            ks, vs = [], []
            for c in range(n_kc):
                src_cols = pl.ds(col0 + c * _LANES, _LANES)
                dst_cols = pl.ds(c * _LANES, _LANES)
                ks.append(pltpu.make_async_copy(
                    k_hbm.at[0, h, :, src_cols], kbuf.at[slot, :, dst_cols], sem_k.at[slot]))
                vs.append(pltpu.make_async_copy(
                    v_hbm.at[0, h, :, src_cols], vbuf.at[slot, :, dst_cols], sem_v.at[slot]))
            return _interleave(ks, vs)

        def wq_descs(p):
            ds = []
            for c in range(pair_w // _LANES):
                for r in range(D // wq_rows):
                    rows = pl.ds(r * wq_rows, wq_rows)
                    cstart = p * pair_w + c * _LANES
                    if not isinstance(cstart, int):
                        cstart = pl.multiple_of(cstart, _LANES)
                    ds.append(pltpu.make_async_copy(
                        wq_hbm.at[rows, pl.ds(cstart, _LANES)],
                        wqbuf.at[rows, pl.ds(c * _LANES, _LANES)], sem_wq.at[0]))
            return ds

        def wo_descs(p):
            ds = []
            for c in range(D // _LANES):
                for r in range(2):
                    rstart = p * pair_w + r * _DH
                    if not isinstance(rstart, int):
                        rstart = pl.multiple_of(rstart, 64)
                    cols = pl.ds(c * _LANES, _LANES)
                    ds.append(pltpu.make_async_copy(
                        wo_hbm.at[pl.ds(rstart, _DH), cols],
                        wobuf.at[pl.ds(r * _DH, _DH), cols], sem_wo.at[0]))
            return ds

        def w1_descs():
            ds = []
            for c in range(F // _LANES):
                for r in range(D // wq_rows):
                    rows = pl.ds(r * wq_rows, wq_rows)
                    cols = pl.ds(c * _LANES, _LANES)
                    ds.append(pltpu.make_async_copy(
                        w1_hbm.at[rows, cols], w1buf.at[rows, cols], sem_w1.at[0]))
            return ds

        def w2_descs():
            ds = []
            for rp in range(w2_blocks // 2):
                for c in range(D // _LANES):
                    for r in (2 * rp, 2 * rp + 1):
                        rows = pl.ds(r * _DH, _DH)
                        cols = pl.ds(c * _LANES, _LANES)
                        ds.append(pltpu.make_async_copy(
                            w2_hbm.at[rows, cols], w2buf.at[rows, cols], sem_w2.at[rp]))
            return ds

        def wait_full(buf, sem):
            pltpu.make_async_copy(buf, buf, sem).wait()

        small = [
            pltpu.make_async_copy(x_hbm, xbuf, sem_s.at[0]),
            pltpu.make_async_copy(b1_hbm, b1buf, sem_s.at[1]),
            pltpu.make_async_copy(b2_hbm, b2buf, sem_s.at[2]),
            pltpu.make_async_copy(gw_hbm, gwbuf, sem_s.at[3]),
        ]

        _start_all(small)
        _start_all(w1_descs())
        _start_all(wq_descs(0))
        _start_all(kv_descs(0, 0))

        for d in small:
            d.wait()
        x = xbuf[0]
        x8 = jnp.broadcast_to(x.astype(_F32), (8, D)).astype(_BF16)
        gate = jax.nn.sigmoid(jnp.sum(
            x.astype(_F32) * gwbuf[...].reshape(1, D).astype(_F32), axis=-1, keepdims=True))
        wait_full(w1buf, sem_w1.at[0])
        hid = jnp.dot(x8, w1buf[...], preferred_element_type=_F32)
        hid = hid + b1buf[...].reshape(1, F).astype(_F32)
        hid = jax.nn.gelu(hid, approximate=True).astype(_BF16)

        def attend(q, slot):
            s = jnp.dot(q, kbuf[slot], preferred_element_type=_F32) * scale
            m = jnp.max(s, axis=-1, keepdims=True)
            p = jnp.exp(s - m)
            l = jnp.sum(p, axis=-1, keepdims=True)
            o = jax.lax.dot_general(p.astype(_BF16), vbuf[slot], (((1,), (1,)), ((), ())),
                                    preferred_element_type=_F32)
            return (o / l).astype(_BF16)

        def pair_step(p, acc):
            _start_all(wo_descs(p))
            _start_all(kv_descs(2 * p + 1, 1))

            wait_full(wqbuf, sem_wq.at[0])
            q2 = jnp.dot(x8, wqbuf[...], preferred_element_type=_F32).astype(_BF16)
            wait_full(kbuf.at[0], sem_k.at[0])
            wait_full(vbuf.at[0], sem_v.at[0])
            o_a = attend(q2[:, :_DH], 0)

            @pl.when(p + 1 < n_pairs)
            def _():
                _start_all(wq_descs(p + 1))
                _start_all(kv_descs(2 * p + 2, 0))

            @pl.when(p + 1 == n_pairs)
            def _():
                _start_all(w2_descs())

            wait_full(wobuf, sem_wo.at[0])
            acc = acc + jnp.dot(o_a, wobuf[0:_DH, :], preferred_element_type=_F32)
            wait_full(kbuf.at[1], sem_k.at[1])
            wait_full(vbuf.at[1], sem_v.at[1])
            o_b = attend(q2[:, _DH:], 1)
            acc = acc + jnp.dot(o_b, wobuf[_DH:pair_w, :], preferred_element_type=_F32)
            return acc

        att = jax.lax.fori_loop(0, n_pairs, pair_step, jnp.zeros((8, D), _F32))

        mlp = jnp.broadcast_to(b2buf[...].reshape(1, D).astype(_F32), (8, D))
        for rp in range(w2_blocks // 2):
            rows = pl.ds(rp * pair_w, pair_w)
            wait_full(w2buf.at[rows], sem_w2.at[rp])
            mlp = mlp + jnp.dot(hid[:, rp * pair_w:(rp + 1) * pair_w], w2buf[rows, :],
                                preferred_element_type=_F32)

        out = gate * att[0:1] + (1.0 - gate) * mlp[0:1]
        o_ref[0] = out.astype(o_ref.dtype)

    return kernel


@jax.jit
def pallas_gated_mix__sliding_block_cached__dense_activation_gelu__decode_kernel(
    A_x: jax.Array,
    A_k_cache: jax.Array,
    A_v_cache: jax.Array,
    A_wq: jax.Array,
    A_wo: jax.Array,
    B_x: jax.Array,
    B_w1: jax.Array,
    B_b1: jax.Array,
    B_w2: jax.Array,
    B_b2: jax.Array,
    gate_w: jax.Array,
):
    del B_x
    B, Sq, D = A_x.shape
    _, Hkv, Sk, Dh = A_k_cache.shape
    F = B_w1.shape[1]
    assert (B, Sq, Hkv, Dh) == (1, 1, _HQ, _DH)
    W = min(4096, max(256, Sk // 4))

    kt = jnp.swapaxes(A_k_cache, 2, 3)
    vt = jnp.swapaxes(A_v_cache, 2, 3)

    dma = pltpu.SemaphoreType.DMA
    return pl.pallas_call(
        _make_kernel(D, F, Sk, W),
        out_shape=jax.ShapeDtypeStruct((B, Sq, D), A_x.dtype),
        in_specs=[pl.BlockSpec(memory_space=pl.ANY)] * 10,
        out_specs=pl.BlockSpec(memory_space=pltpu.VMEM),
        scratch_shapes=[
            pltpu.VMEM((2, _DH, W), _BF16),
            pltpu.VMEM((2, _DH, W), _BF16),
            pltpu.VMEM((D, 2 * _DH), _BF16),
            pltpu.VMEM((2 * _DH, D), _BF16),
            pltpu.VMEM((D, F), _BF16),
            pltpu.VMEM((F, D), _BF16),
            pltpu.VMEM((1, 1, D), _BF16),
            pltpu.VMEM((F,), _BF16),
            pltpu.VMEM((D,), _BF16),
            pltpu.VMEM((D,), _BF16),
            dma((2,)), dma((2,)), dma((1,)), dma((1,)), dma((1,)), dma((4,)), dma((4,)),
        ],
        compiler_params=pltpu.CompilerParams(vmem_limit_bytes=48 * 1024 * 1024),
    )(A_x, kt, vt, A_wq, A_wo, B_w1, B_b1, B_w2, B_b2, gate_w)
```

```python
import jax
import jax.numpy as jnp
import jax.experimental.pallas as pl
import jax.experimental.pallas.tpu as pltpu

_F32 = jnp.float32
_BF16 = jnp.bfloat16
_LANES = 128

_HQ = 32
_DH = 192

_QK_COLS = 512
_PV_COLS = 512
_K_WAIT_SLOT = 8
_N_VSLOT = 4
_N_WOSLOT = 4
_W2_SPLIT = (384, 384, 384, 384)
_N_SEMS = 2 + _N_VSLOT + len(_W2_SPLIT)


def _make_kernel(D, F, Sk, W):
    scale = _DH ** -0.5
    n_pairs = _HQ // 2
    pair_w = 2 * _DH
    col0 = Sk - W
    col_shape = (D // 4, _LANES)
    row_shape = (32, D)
    half_f = F // 2

    def body(x_hbm, k_hbm, v_hbm, wq_hbm, wo_hbm, w1_hbm, b1_hbm, w2_hbm, b2_hbm, gw_hbm,
             kbuf, vbuf, wqbuf, wobuf, w1buf, w2buf, xbuf, b1buf, b2buf, gwbuf, obuf, sems):

        def sem_k(i):
            return sems.at[i]

        def sem_v(i):
            return sems.at[2 + i]

        def sem_w2(i):
            return sems.at[2 + _N_VSLOT + i]

        def mod(a, n):
            return a % n if isinstance(a, int) else jax.lax.rem(a, n)

        def tiles(src, dst, r0, c0, n_rows, n_cols, shape, sem, col_major=False):
            tr, tc = shape
            idx = [(r, c) for r in range(n_rows // tr) for c in range(n_cols // tc)]
            if col_major:
                idx.sort(key=lambda rc: (rc[1], rc[0]))
            makers = []
            for r, c in idx:
                rs = r0 + r * tr
                cs = c0 + c * tc
                if not isinstance(rs, int):
                    rs = pl.multiple_of(rs, 32)
                if not isinstance(cs, int):
                    cs = pl.multiple_of(cs, _LANES)

                def make(rs=rs, cs=cs, r=r, c=c):
                    return pltpu.make_async_copy(
                        src.at[pl.ds(rs, tr), pl.ds(cs, tc)],
                        dst.at[pl.ds(r * tr, tr), pl.ds(c * tc, tc)], sem)

                makers.append(make)
            return makers

        def k_copies(h, slot):
            return tiles(k_hbm.at[0, h], kbuf.at[slot], 0, col0, _DH, W, (_DH, _LANES),
                         sem_k(slot))

        def v_copies(h):
            slot = mod(h, _N_VSLOT)
            return tiles(v_hbm.at[0, h], vbuf.at[slot], 0, col0, _DH, W, (_DH, _LANES),
                         sem_v(slot))

        def wq_copies(p):
            return tiles(wq_hbm, wqbuf, 0, p * pair_w, D, pair_w, col_shape, sem_k(0), True)

        def wo_copies(p):
            return tiles(wo_hbm, wobuf.at[mod(p, _N_WOSLOT)], p * pair_w, 0, pair_w, D,
                         row_shape, sem_v(mod(2 * p, _N_VSLOT)))

        def a_even(p):
            return wq_copies(p) + k_copies(2 * p, 0)

        def a_odd(p):
            return k_copies(2 * p + 1, 1)

        def b_even(p):
            return v_copies(2 * p) + wo_copies(p)

        def b_odd(p):
            return v_copies(2 * p + 1)

        w1_lo = w1buf.at[:, pl.ds(0, half_f)]
        w1_hi = w1buf.at[:, pl.ds(half_f, half_f)]
        w1_a = tiles(w1_hbm, w1_lo, 0, 0, D, half_f, col_shape, sem_k(1), True)
        w1_b = tiles(w1_hbm, w1_hi, 0, half_f, D, half_f, col_shape, sem_v(_N_VSLOT - 1), True)
        w2_a, w2_b = [], []
        r0 = 0
        for i, rows in enumerate(_W2_SPLIT):
            t = tiles(w2_hbm, w2buf.at[pl.ds(r0, rows)], r0, 0, rows, D, row_shape, sem_w2(i))
            w2_a += t[:len(t) // 2]
            w2_b += t[len(t) // 2:]
            r0 += rows

        def wait_full(buf, sem):
            pltpu.make_async_copy(buf, buf, sem).wait()

        def run(a, b, pieces):
            n = max(len(a), len(b), (max(pieces) + 1) if pieces else 0)
            for i in range(n):
                if i < len(b):
                    b[i]().start(priority=1)
                if i < len(a):
                    a[i]().start(priority=0)
                for fn in pieces.get(i, ()):
                    fn()

        small = [
            pltpu.make_async_copy(x_hbm, xbuf, sem_k(1)),
            pltpu.make_async_copy(b1_hbm, b1buf, sem_k(1)),
            pltpu.make_async_copy(b2_hbm, b2buf, sem_k(1)),
            pltpu.make_async_copy(gw_hbm, gwbuf, sem_k(1)),
        ]

        b_1 = b_odd(0)
        n_pre = len(b_1) - len(w1_a)
        for make in w1_b + b_even(0) + b_1[:n_pre]:
            make().start(priority=1)
        for cp in small:
            cp.start()
        run(w1_a, b_1[n_pre:], {})

        st = {}

        def piece_x():
            for cp in small:
                cp.wait()
            wait_full(w1_lo, sem_k(1))
            wait_full(w1_hi, sem_v(_N_VSLOT - 1))
            x = xbuf[0].astype(_F32)
            st['x8'] = jnp.broadcast_to(x, (8, D)).astype(_BF16)
            st['gate'] = jax.nn.sigmoid(jnp.sum(
                x * gwbuf[...].reshape(1, D).astype(_F32), axis=-1, keepdims=True))
            st['hid'] = []

        def piece_hid(c):
            def fn():
                cols = slice(c * 256, (c + 1) * 256)
                hid = jnp.dot(st['x8'], w1buf[:, cols], preferred_element_type=_F32)
                hid = hid + b1buf[...].reshape(1, F)[:, cols].astype(_F32)
                st['hid'].append(jax.nn.gelu(hid, approximate=True).astype(_BF16))
            return fn

        pieces = {10: [piece_x]}
        for c in range(F // 256):
            pieces[11 + 2 * c] = [piece_hid(c)]
        run(a_even(0), b_even(1), pieces)
        x8 = st['x8']
        gate = st['gate']
        hid = jnp.concatenate(st['hid'], axis=1)

        def head_pieces(h, p, first, st):
            pcs = {}
            pos = [_K_WAIT_SLOT]

            def add(fn, adv=1):
                pcs.setdefault(pos[0], []).append(fn)
                pos[0] += adv

            kslot = 0 if first else 1
            vslot = mod(h, _N_VSLOT)
            wslot = mod(p, _N_WOSLOT)

            def wait_k():
                wait_full(kbuf.at[kslot], sem_k(kslot))
                if first:
                    wait_full(wqbuf, sem_k(kslot))
                st['s'] = []
                st['qs'] = []
            add(wait_k, 0)

            if first:
                for c in range(pair_w // _LANES):
                    def q_proj(c=c):
                        st['qs'].append(jnp.dot(
                            x8, wqbuf[:, c * _LANES:(c + 1) * _LANES],
                            preferred_element_type=_F32).astype(_BF16))
                        if c == pair_w // _LANES - 1:
                            st['q2'] = jnp.concatenate(st['qs'], axis=1)
                    add(q_proj)

            for c in range(W // _QK_COLS):
                def qk(c=c):
                    q = st['q2'][:, :_DH] if first else st['q2'][:, _DH:]
                    st['s'].append(jnp.dot(
                        q, kbuf[kslot, :, c * _QK_COLS:(c + 1) * _QK_COLS],
                        preferred_element_type=_F32))
                add(qk)

            def row_max():
                s = jnp.concatenate(st['s'], axis=1) * scale
                st['sc'] = s
                st['m'] = jnp.max(s, axis=-1, keepdims=True)
            add(row_max)

            def exps():
                e = jnp.exp(st['sc'] - st['m'])
                st['l'] = jnp.sum(e, axis=-1, keepdims=True)
                st['p'] = e.astype(_BF16)
            add(exps)

            def wait_v():
                wait_full(vbuf.at[vslot], sem_v(vslot))
                if first:
                    wait_full(wobuf.at[wslot], sem_v(vslot))
                st['o'] = None
            add(wait_v, 0)

            for c in range(W // _PV_COLS):
                def pv(c=c):
                    cols = slice(c * _PV_COLS, (c + 1) * _PV_COLS)
                    t = jax.lax.dot_general(
                        st['p'][:, cols], vbuf[vslot, :, cols], (((1,), (1,)), ((), ())),
                        preferred_element_type=_F32)
                    st['o'] = t if st['o'] is None else st['o'] + t
                add(pv)

            def out_proj():
                o = (st['o'] / st['l']).astype(_BF16)
                rows = slice(0, _DH) if first else slice(_DH, pair_w)
                st['acc'] = st['acc'] + jnp.dot(
                    o, wobuf[wslot, rows, :], preferred_element_type=_F32)
            add(out_proj)
            return pcs

        def pair_step(p, acc, left=2):
            st = {'acc': acc}
            run(a_odd(p), b_odd(p + 1) if left >= 1 else [],
                head_pieces(2 * p, p, True, st))
            if left == 2:
                a, b = a_even(p + 1), b_even(p + 2)
            elif left == 1:
                a, b = a_even(p + 1), w2_b
            else:
                a, b = w2_a, []
            run(a, b, head_pieces(2 * p + 1, p, False, st))
            return st['acc']

        acc = jax.lax.fori_loop(0, n_pairs - 2, pair_step, jnp.zeros((8, D), _F32))
        acc = pair_step(n_pairs - 2, acc, 1)
        att = pair_step(n_pairs - 1, acc, 0)

        mlp = jnp.broadcast_to(b2buf[...].reshape(1, D).astype(_F32), (8, D))
        r0 = 0
        for i, rows in enumerate(_W2_SPLIT):
            wait_full(w2buf.at[pl.ds(r0, rows)], sem_w2(i))
            mlp = mlp + jnp.dot(hid[:, r0:r0 + rows], w2buf[r0:r0 + rows, :],
                                preferred_element_type=_F32)
            r0 += rows

        out = gate * att[0:1] + (1.0 - gate) * mlp[0:1]
        obuf[0] = out.astype(obuf.dtype)

    def kernel(*refs):
        ins, o_hbm, scratch, out_sem = refs[:10], refs[10], refs[11:22], refs[22]
        out_copy = pltpu.make_async_copy(scratch[-1], o_hbm, out_sem.at[0])

        def scoped(sems):
            body(*ins, *scratch, sems)
            out_copy.start()

        pl.run_scoped(scoped, pltpu.SemaphoreType.DMA((_N_SEMS,)))
        out_copy.wait()

    return kernel


@jax.jit
def pallas_gated_mix__sliding_block_cached__dense_activation_gelu__decode_kernel(
    A_x: jax.Array,
    A_k_cache: jax.Array,
    A_v_cache: jax.Array,
    A_wq: jax.Array,
    A_wo: jax.Array,
    B_x: jax.Array,
    B_w1: jax.Array,
    B_b1: jax.Array,
    B_w2: jax.Array,
    B_b2: jax.Array,
    gate_w: jax.Array,
):
    del B_x
    B, Sq, D = A_x.shape
    _, Hkv, Sk, Dh = A_k_cache.shape
    F = B_w1.shape[1]
    assert (B, Sq, Hkv, Dh) == (1, 1, _HQ, _DH)
    assert sum(_W2_SPLIT) == F
    W = min(4096, max(256, Sk // 4))

    kt = jnp.swapaxes(A_k_cache, 2, 3)
    vt = jnp.swapaxes(A_v_cache, 2, 3)

    return pl.pallas_call(
        _make_kernel(D, F, Sk, W),
        out_shape=jax.ShapeDtypeStruct((B, Sq, D), A_x.dtype),
        in_specs=[pl.BlockSpec(memory_space=pl.ANY)] * 10,
        out_specs=pl.BlockSpec(memory_space=pl.ANY),
        scratch_shapes=[
            pltpu.VMEM((2, _DH, W), _BF16),
            pltpu.VMEM((_N_VSLOT, _DH, W), _BF16),
            pltpu.VMEM((D, 2 * _DH), _BF16),
            pltpu.VMEM((_N_WOSLOT, 2 * _DH, D), _BF16),
            pltpu.VMEM((D, F), _BF16),
            pltpu.VMEM((F, D), _BF16),
            pltpu.VMEM((1, 1, D), _BF16),
            pltpu.VMEM((F,), _BF16),
            pltpu.VMEM((D,), _BF16),
            pltpu.VMEM((D,), _BF16),
            pltpu.VMEM((1, 1, D), _BF16),
            pltpu.SemaphoreType.DMA((1,)),
        ],
        compiler_params=pltpu.CompilerParams(vmem_limit_bytes=64 * 1024 * 1024),
    )(A_x, kt, vt, A_wq, A_wo, B_w1, B_b1, B_w2, B_b2, gate_w)
```

```python
import jax
import jax.numpy as jnp
import jax.experimental.pallas as pl
import jax.experimental.pallas.tpu as pltpu

_F32 = jnp.float32
_BF16 = jnp.bfloat16
_LANES = 128

_HQ = 32
_DH = 192

_LEAD = 25
_PHASE_A, _PHASE_B = 0.25, 0.75
_W2_GROUPS = ((640, 'a'), (512, 'b'), (256, 'b'), (128, 'b'))

_SEM_K, _SEM_V, _SEM_WO, _SEM_WQ, _SEM_W1, _SEM_SMALL, _SEM_W2 = 0, 2, 4, 6, 7, 8, 12
_N_SEMS = _SEM_W2 + len(_W2_GROUPS)


def _spread(main, extra, phase):
    out, j = [], 0
    for i, item in enumerate(main):
        out.append(item)
        while j < len(extra) and (j + phase) / len(extra) <= (i + 1) / len(main):
            out.append(extra[j])
            j += 1
    return out + extra[j:]


def _halves(items):
    return items[:len(items) // 2], items[len(items) // 2:]


def _make_kernel(D, F, Sk, W):
    scale = _DH ** -0.5
    n_pairs = _HQ // 2
    pair_w = 2 * _DH
    col0 = Sk - W
    kv_chunk = (_DH // 2, _LANES)
    wq_chunk = (8, _HQ * _DH // 2)
    w1_chunk = (16, F)
    row_chunk = (32, D)

    def body(x_hbm, k_hbm, v_hbm, wq_hbm, wo_hbm, w1_hbm, b1_hbm, w2_hbm, b2_hbm, gw_hbm,
             kbuf, vbuf, wqbuf, wobuf, w1buf, w2buf, xbuf, b1buf, b2buf, gwbuf, obuf, sems):

        def tiles(src, dst, r0, c0, n_rows, n_cols, shape, sem, dst_r0=0):
            tr, tc = shape
            makers = []
            for r in range(n_rows // tr):
                for c in range(n_cols // tc):
                    rs = r0 + r * tr
                    if not isinstance(rs, int):
                        rs = pl.multiple_of(rs, 32)

                    def make(rs=rs, r=r, c=c):
                        return pltpu.make_async_copy(
                            src.at[pl.ds(rs, tr), pl.ds(c0 + c * tc, tc)],
                            dst.at[pl.ds(dst_r0 + r * tr, tr), pl.ds(c * tc, tc)],
                            sems.at[sem])

                    makers.append(make)
            return makers

        def k_block(h, s):
            return _halves(tiles(k_hbm.at[0, h], kbuf.at[s], 0, col0, _DH, W, kv_chunk,
                                 _SEM_K + s))

        def v_block(h, s):
            a, b = _halves(tiles(v_hbm.at[0, h], vbuf.at[s], 0, col0, _DH, W, kv_chunk,
                                 _SEM_V + s))
            wa, wb = _halves(tiles(wo_hbm, wobuf.at[s], h * _DH, 0, _DH, D, row_chunk,
                                   _SEM_WO + s))
            return _spread(a, wa, _PHASE_A), _spread(b, wb, _PHASE_B)

        wq_a, wq_b = _halves(tiles(wq_hbm, wqbuf, 0, 0, D, _HQ * _DH, wq_chunk, _SEM_WQ))
        w1_a, w1_b = _halves(tiles(w1_hbm, w1buf, 0, 0, D, F, w1_chunk, _SEM_W1))
        w2_a, w2_b = [], []
        r0 = 0
        for i, (rows, stream) in enumerate(_W2_GROUPS):
            group = tiles(w2_hbm, w2buf, r0, 0, rows, D, row_chunk, _SEM_W2 + i, r0)
            (w2_a if stream == 'a' else w2_b).extend(group)
            r0 += rows

        def wait_full(buf, sem):
            pltpu.make_async_copy(buf, buf, sems.at[sem]).wait()

        def issue(a, b):
            for i in range(max(len(a), len(b))):
                if i < len(b):
                    b[i]().start(priority=1)
                if i < len(a):
                    a[i]().start(priority=0)

        small = [
            pltpu.make_async_copy(src, dst, sems.at[_SEM_SMALL + i])
            for i, (src, dst) in enumerate(
                ((x_hbm, xbuf), (b1_hbm, b1buf), (b2_hbm, b2buf), (gw_hbm, gwbuf)))
        ]

        k0a, k0b = k_block(0, 0)
        v0a, v0b = v_block(0, 0)
        pro_a = _spread(w1_a + wq_a, k0a + v0a, _PHASE_A)
        pro_b = _spread(w1_b + wq_b, k0b + v0b, _PHASE_B) + k_block(1, 1)[1][:_LEAD]
        issue([], pro_b[:_LEAD])
        for cp in small:
            cp.start()
        issue(pro_a, pro_b[_LEAD:])

        def scores(q, s):
            wait_full(kbuf.at[s], _SEM_K + s)
            sc = jnp.dot(q, kbuf[s], preferred_element_type=_F32) * scale
            e = jnp.exp(sc - jnp.max(sc, axis=-1, keepdims=True))
            return e.astype(_BF16), jnp.sum(e, axis=-1, keepdims=True)

        def project(e, l, s, acc):
            wait_full(vbuf.at[s], _SEM_V + s)
            wait_full(wobuf.at[s], _SEM_WO + s)
            o = jax.lax.dot_general(e, vbuf[s], (((1,), (1,)), ((), ())),
                                    preferred_element_type=_F32)
            return acc + jnp.dot((o / l).astype(_BF16), wobuf[s],
                                 preferred_element_type=_F32)

        st = {}

        def pair_step(p, acc, first=False, last=False):
            h = 2 * p
            k1a, k1b = k_block(h + 1, 1)
            v1a, v1b = v_block(h + 1, 1)
            if not last:
                k2a, k2b = k_block(h + 2, 0)
                v2a, v2b = v_block(h + 2, 0)
                k3b = k_block(h + 3, 1)[1]

            issue(k1a, k1b[_LEAD:] + v1b[:_LEAD])
            if first:
                for cp in small:
                    cp.wait()
                wait_full(wqbuf, _SEM_WQ)
                x = xbuf[0].astype(_F32)
                st['x8'] = jnp.broadcast_to(x, (8, D)).astype(_BF16)
                st['gate'] = jax.nn.sigmoid(jnp.sum(
                    x * gwbuf[...].reshape(1, D).astype(_F32), axis=-1, keepdims=True))
            c0 = p * pair_w
            if not isinstance(c0, int):
                c0 = pl.multiple_of(c0, _LANES)
            q2 = jnp.dot(st['x8'], wqbuf[:, pl.ds(c0, pair_w)],
                         preferred_element_type=_F32).astype(_BF16)
            e, l = scores(q2[:, :_DH], 0)

            issue(v1a, v1b[_LEAD:] + (w2_b if last else k2b)[:_LEAD])
            acc = project(e, l, 0, acc)

            if not last:
                issue(k2a, k2b[_LEAD:] + v2b[:_LEAD])
            e, l = scores(q2[:, _DH:], 1)

            if last:
                issue(w2_a, w2_b[_LEAD:])
            else:
                issue(v2a, v2b[_LEAD:] + k3b[:_LEAD])
            acc = project(e, l, 1, acc)

            if first:
                wait_full(w1buf, _SEM_W1)
                hid = jnp.dot(st['x8'], w1buf[...], preferred_element_type=_F32)
                hid = hid + b1buf[...].reshape(1, F).astype(_F32)
                st['hid'] = jax.nn.gelu(hid, approximate=True).astype(_BF16)
            return acc

        acc = pair_step(0, jnp.zeros((8, D), _F32), first=True)
        acc = jax.lax.fori_loop(1, n_pairs - 1, pair_step, acc)
        att = pair_step(n_pairs - 1, acc, last=True)

        mlp = jnp.broadcast_to(b2buf[...].reshape(1, D).astype(_F32), (8, D))
        r0 = 0
        for i, (rows, _) in enumerate(_W2_GROUPS):
            wait_full(w2buf.at[pl.ds(r0, rows)], _SEM_W2 + i)
            mlp = mlp + jnp.dot(st['hid'][:, r0:r0 + rows], w2buf[r0:r0 + rows, :],
                                preferred_element_type=_F32)
            r0 += rows

        gate = st['gate']
        out = gate * att[0:1] + (1.0 - gate) * mlp[0:1]
        obuf[0] = out.astype(obuf.dtype)

    def kernel(*refs):
        ins, o_hbm, scratch, out_sem = refs[:10], refs[10], refs[11:22], refs[22]
        out_copy = pltpu.make_async_copy(scratch[-1], o_hbm, out_sem.at[0])

        def scoped(sems):
            body(*ins, *scratch, sems)
            out_copy.start()

        pl.run_scoped(scoped, pltpu.SemaphoreType.DMA((_N_SEMS,)))
        out_copy.wait()

    return kernel


@jax.jit
def pallas_gated_mix__sliding_block_cached__dense_activation_gelu__decode_kernel(
    A_x: jax.Array,
    A_k_cache: jax.Array,
    A_v_cache: jax.Array,
    A_wq: jax.Array,
    A_wo: jax.Array,
    B_x: jax.Array,
    B_w1: jax.Array,
    B_b1: jax.Array,
    B_w2: jax.Array,
    B_b2: jax.Array,
    gate_w: jax.Array,
):
    del B_x
    B, Sq, D = A_x.shape
    _, Hkv, Sk, Dh = A_k_cache.shape
    F = B_w1.shape[1]
    assert (B, Sq, Hkv, Dh) == (1, 1, _HQ, _DH)
    assert sum(rows for rows, _ in _W2_GROUPS) == F
    W = min(4096, max(256, Sk // 4))

    kt = jnp.swapaxes(A_k_cache, 2, 3)
    vt = jnp.swapaxes(A_v_cache, 2, 3)

    return pl.pallas_call(
        _make_kernel(D, F, Sk, W),
        out_shape=jax.ShapeDtypeStruct((B, Sq, D), A_x.dtype),
        in_specs=[pl.BlockSpec(memory_space=pl.ANY)] * 10,
        out_specs=pl.BlockSpec(memory_space=pl.ANY),
        scratch_shapes=[
            pltpu.VMEM((2, _DH, W), _BF16),
            pltpu.VMEM((2, _DH, W), _BF16),
            pltpu.VMEM((D, _HQ * _DH), _BF16),
            pltpu.VMEM((2, _DH, D), _BF16),
            pltpu.VMEM((D, F), _BF16),
            pltpu.VMEM((F, D), _BF16),
            pltpu.VMEM((1, 1, D), _BF16),
            pltpu.VMEM((F,), _BF16),
            pltpu.VMEM((D,), _BF16),
            pltpu.VMEM((D,), _BF16),
            pltpu.VMEM((1, 1, D), _BF16),
            pltpu.SemaphoreType.DMA((1,)),
        ],
        compiler_params=pltpu.CompilerParams(vmem_limit_bytes=64 * 1024 * 1024),
    )(A_x, kt, vt, A_wq, A_wo, B_w1, B_b1, B_w2, B_b2, gate_w)
```

```python
import jax
import jax.numpy as jnp
import jax.experimental.pallas as pl
import jax.experimental.pallas.tpu as pltpu

_F32 = jnp.float32
_BF16 = jnp.bfloat16
_LANES = 128

_HQ = 32
_DH = 192

_LEAD = 25
_PHASE_A, _PHASE_B = 0.25, 0.75
_W2_EARLY, _W2_LATE, _W2_TAIL = 768, 512, (192, 64)

_SEM_K, _SEM_V, _SEM_WO, _SEM_WQ, _SEM_W1, _SEM_SMALL, _SEM_W2 = 0, 2, 4, 6, 7, 8, 12
_N_SEMS = _SEM_W2 + 2 + len(_W2_TAIL)


def _spread(main, extra, phase):
    out, j = [], 0
    for i, item in enumerate(main):
        out.append(item)
        while j < len(extra) and (j + phase) / len(extra) <= (i + 1) / len(main):
            out.append(extra[j])
            j += 1
    return out + extra[j:]


def _halves(items):
    return items[:len(items) // 2], items[len(items) // 2:]


def _make_kernel(D, F, Sk, W):
    scale = _DH ** -0.5
    n_pairs = _HQ // 2
    pair_w = 2 * _DH
    col0 = Sk - W
    kv_chunk = (_DH // 2, _LANES)
    wq_chunk = (8, _HQ * _DH // 2)
    w1_chunk = (16, F)
    row_chunk = (32, D)
    tail_rows = sum(_W2_TAIL)
    tail0 = F - tail_rows

    def body(x_hbm, k_hbm, v_hbm, wq_hbm, wo_hbm, w1_hbm, b1_hbm, w2_hbm, b2_hbm, gw_hbm,
             kbuf, vbuf, wqbuf, wobuf, w1buf, w2buf, xbuf, b1buf, b2buf, gwbuf, obuf, sems):

        def tiles(src, dst, r0, c0, n_rows, n_cols, shape, sem, dst_r0=0):
            tr, tc = shape
            makers = []
            for r in range(n_rows // tr):
                for c in range(n_cols // tc):
                    rs = r0 + r * tr
                    if not isinstance(rs, int):
                        rs = pl.multiple_of(rs, 32)

                    def make(rs=rs, r=r, c=c):
                        return pltpu.make_async_copy(
                            src.at[pl.ds(rs, tr), pl.ds(c0 + c * tc, tc)],
                            dst.at[pl.ds(dst_r0 + r * tr, tr), pl.ds(c * tc, tc)],
                            sems.at[sem])

                    makers.append(make)
            return makers

        def block(src, dst, sem, extra_a, extra_b):
            a, b = _halves(tiles(src, dst, 0, col0, _DH, W, kv_chunk, sem))
            return _spread(a, extra_a, _PHASE_A), _spread(b, extra_b, _PHASE_B)

        def k_block(h, s, extra=([], [])):
            return block(k_hbm.at[0, h], kbuf.at[s], _SEM_K + s, *extra)

        def v_block(h, s, extra=([], [])):
            wa, wb = _halves(tiles(wo_hbm, wobuf.at[s], h * _DH, 0, _DH, D, row_chunk,
                                   _SEM_WO + s))
            return block(v_hbm.at[0, h], vbuf.at[s], _SEM_V + s, wa + extra[0], wb + extra[1])

        def w2_rows(r0, rows, group):
            return tiles(w2_hbm, w2buf, r0, 0, rows, D, row_chunk, _SEM_W2 + group, r0)

        wq_a, wq_b = _halves(tiles(wq_hbm, wqbuf, 0, 0, D, _HQ * _DH, wq_chunk, _SEM_WQ))
        w1_a, w1_b = _halves(tiles(w1_hbm, w1buf, 0, 0, D, F, w1_chunk, _SEM_W1))
        w2e_a, w2e_b = _halves(w2_rows(0, _W2_EARLY, 0))
        w2_end = w2_rows(_W2_EARLY, _W2_LATE, 1)
        r0 = tail0
        for i, rows in enumerate(_W2_TAIL):
            w2_end += w2_rows(r0, rows, 2 + i)
            r0 += rows
        assert len(w2_end) <= _LEAD

        mlp_a, mlp_b = w1_a + w2e_a, w1_b + w2e_b
        n_wo = _DH // row_chunk[0] // 2
        per = (len(mlp_a) + 2 * n_wo) / 4
        cuts = [0, round(per), round(2 * per - n_wo), round(3 * per - n_wo), len(mlp_a)]
        riders = [(mlp_a[cuts[i]:cuts[i + 1]], mlp_b[cuts[i]:cuts[i + 1]]) for i in range(4)]
        no_riders = [([], [])] * 4

        def wait_full(buf, sem):
            pltpu.make_async_copy(buf, buf, sems.at[sem]).wait()

        def issue(a, b):
            for i in range(max(len(a), len(b))):
                if i < len(b):
                    b[i]().start(priority=1)
                if i < len(a):
                    a[i]().start(priority=0)

        small = [
            pltpu.make_async_copy(src, dst, sems.at[_SEM_SMALL + i])
            for i, (src, dst) in enumerate(
                ((x_hbm, xbuf), (b1_hbm, b1buf), (b2_hbm, b2buf), (gw_hbm, gwbuf)))
        ]

        k0a, k0b = k_block(0, 0)
        v0a, v0b = v_block(0, 0)
        pro_a = _spread(wq_a, k0a + v0a, _PHASE_A)
        pro_b = _spread(wq_b, k0b + v0b, _PHASE_B) + k_block(1, 1, riders[0])[1][:_LEAD]
        issue([], pro_b[:_LEAD])
        for cp in small:
            cp.start()
        issue(pro_a, pro_b[_LEAD:])

        def scores(q, s):
            wait_full(kbuf.at[s], _SEM_K + s)
            sc = jnp.dot(q, kbuf[s], preferred_element_type=_F32) * scale
            e = jnp.exp(sc - jnp.max(sc, axis=-1, keepdims=True))
            return e.astype(_BF16), jnp.sum(e, axis=-1, keepdims=True)

        def project(e, l, s, acc):
            wait_full(vbuf.at[s], _SEM_V + s)
            wait_full(wobuf.at[s], _SEM_WO + s)
            o = jax.lax.dot_general(e, vbuf[s], (((1,), (1,)), ((), ())),
                                    preferred_element_type=_F32)
            return acc + jnp.dot((o / l).astype(_BF16), wobuf[s],
                                 preferred_element_type=_F32)

        def w2_matvec(hid, r0, rows, group):
            wait_full(w2buf.at[pl.ds(r0, rows)], _SEM_W2 + group)
            return jnp.dot(hid[:, r0:r0 + rows], w2buf[r0:r0 + rows, :],
                           preferred_element_type=_F32)

        st = {}

        def pair_step(p, acc, first=False, last=False):
            h = 2 * p
            extra = riders if first else no_riders
            k1a, k1b = k_block(h + 1, 1, extra[0])
            v1a, v1b = v_block(h + 1, 1, extra[1])
            if not last:
                k2a, k2b = k_block(h + 2, 0, extra[2])
                v2a, v2b = v_block(h + 2, 0, extra[3])
                k3b = k_block(h + 3, 1)[1]

            issue(k1a, k1b[_LEAD:] + v1b[:_LEAD])
            if first:
                for cp in small:
                    cp.wait()
                wait_full(wqbuf, _SEM_WQ)
                x = xbuf[0].astype(_F32)
                st['x8'] = jnp.broadcast_to(x, (8, D)).astype(_BF16)
                st['gate'] = jax.nn.sigmoid(jnp.sum(
                    x * gwbuf[...].reshape(1, D).astype(_F32), axis=-1, keepdims=True))
            if last:
                wait_full(w1buf, _SEM_W1)
                hid = jnp.dot(st['x8'], w1buf[...], preferred_element_type=_F32)
                hid = hid + b1buf[...].reshape(1, F).astype(_F32)
                hid = jax.nn.gelu(hid, approximate=True).astype(_BF16)
                st['hid'] = hid
                tail = hid[0:1, tail0:].astype(_F32) * (1.0 - st['gate'])
                st['hcol'] = jnp.broadcast_to(tail, (_LANES, tail_rows)).T
            c0 = p * pair_w
            if not isinstance(c0, int):
                c0 = pl.multiple_of(c0, _LANES)
            q2 = jnp.dot(st['x8'], wqbuf[:, pl.ds(c0, pair_w)],
                         preferred_element_type=_F32).astype(_BF16)
            e, l = scores(q2[:, :_DH], 0)

            if last:
                b_end = v1b[_LEAD:] + w2_end
                half = len(v1a) // 2
                issue(v1a[:half], b_end[:half])
                acc = project(e, l, 0, acc)
                st['mlp'] = (b2buf[...].reshape(1, D).astype(_F32)
                             + w2_matvec(st['hid'], 0, _W2_EARLY, 0))
                issue(v1a[half:], b_end[half:])
                e, l = scores(q2[:, _DH:], 1)
            else:
                issue(v1a, v1b[_LEAD:] + k2b[:_LEAD])
                acc = project(e, l, 0, acc)
                issue(k2a, k2b[_LEAD:] + v2b[:_LEAD])
                e, l = scores(q2[:, _DH:], 1)
                issue(v2a, v2b[_LEAD:] + k3b[:_LEAD])
            return project(e, l, 1, acc)

        acc = pair_step(0, jnp.zeros((8, D), _F32), first=True)
        acc = jax.lax.fori_loop(1, n_pairs - 1, pair_step, acc)
        att = pair_step(n_pairs - 1, acc, last=True)

        gate = st['gate']
        mlp = st['mlp'] + w2_matvec(st['hid'], _W2_EARLY, _W2_LATE, 1)
        base = gate * att + (1.0 - gate) * mlp
        row = jax.lax.broadcasted_iota(jnp.int32, (8, D), 0)
        part = jnp.where(row == 0, base, 0.0)
        r0 = tail0
        for i, rows in enumerate(_W2_TAIL):
            wait_full(w2buf.at[pl.ds(r0, rows)], _SEM_W2 + 2 + i)
            hcol = st['hcol'][r0 - tail0:r0 - tail0 + rows]
            sums = []
            for c in range(D // _LANES):
                w = w2buf[r0:r0 + rows, c * _LANES:(c + 1) * _LANES].astype(_F32)
                sums.append(jnp.sum((w * hcol).reshape(rows // 8, 8, _LANES), axis=0))
            part = part + jnp.concatenate(sums, axis=1)
            r0 += rows
        obuf[0] = jnp.sum(part, axis=0, keepdims=True).astype(obuf.dtype)

    def kernel(*refs):
        ins, o_hbm, scratch, out_sem = refs[:10], refs[10], refs[11:22], refs[22]
        out_copy = pltpu.make_async_copy(scratch[-1], o_hbm, out_sem.at[0])

        def scoped(sems):
            body(*ins, *scratch, sems)
            out_copy.start()

        pl.run_scoped(scoped, pltpu.SemaphoreType.DMA((_N_SEMS,)))
        out_copy.wait()

    return kernel


@jax.jit
def pallas_gated_mix__sliding_block_cached__dense_activation_gelu__decode_kernel(
    A_x: jax.Array,
    A_k_cache: jax.Array,
    A_v_cache: jax.Array,
    A_wq: jax.Array,
    A_wo: jax.Array,
    B_x: jax.Array,
    B_w1: jax.Array,
    B_b1: jax.Array,
    B_w2: jax.Array,
    B_b2: jax.Array,
    gate_w: jax.Array,
):
    del B_x
    B, Sq, D = A_x.shape
    _, Hkv, Sk, Dh = A_k_cache.shape
    F = B_w1.shape[1]
    assert (B, Sq, Hkv, Dh) == (1, 1, _HQ, _DH)
    assert _W2_EARLY + _W2_LATE + sum(_W2_TAIL) == F
    W = min(4096, max(256, Sk // 4))
    assert W // _LANES >= _LEAD

    kt = jnp.swapaxes(A_k_cache, 2, 3)
    vt = jnp.swapaxes(A_v_cache, 2, 3)

    return pl.pallas_call(
        _make_kernel(D, F, Sk, W),
        out_shape=jax.ShapeDtypeStruct((B, Sq, D), A_x.dtype),
        in_specs=[pl.BlockSpec(memory_space=pl.ANY)] * 10,
        out_specs=pl.BlockSpec(memory_space=pl.ANY),
        scratch_shapes=[
            pltpu.VMEM((2, _DH, W), _BF16),
            pltpu.VMEM((2, _DH, W), _BF16),
            pltpu.VMEM((D, _HQ * _DH), _BF16),
            pltpu.VMEM((2, _DH, D), _BF16),
            pltpu.VMEM((D, F), _BF16),
            pltpu.VMEM((F, D), _BF16),
            pltpu.VMEM((1, 1, D), _BF16),
            pltpu.VMEM((F,), _BF16),
            pltpu.VMEM((D,), _BF16),
            pltpu.VMEM((D,), _BF16),
            pltpu.VMEM((1, 1, D), _BF16),
            pltpu.SemaphoreType.DMA((1,)),
        ],
        compiler_params=pltpu.CompilerParams(vmem_limit_bytes=64 * 1024 * 1024),
    )(A_x, kt, vt, A_wq, A_wo, B_w1, B_b1, B_w2, B_b2, gate_w)
```

```python
import math

import jax
import jax.numpy as jnp
import jax.experimental.pallas as pl
import jax.experimental.pallas.tpu as pltpu

_F32 = jnp.float32
_BF16 = jnp.bfloat16
_LANES = 128
_SUB = 8

_HQ = 32
_DH = 192

_LEAD = 25
_ROWS_B = 128
_PHASE_A, _PHASE_B = 0.25, 0.75
_GROUP_TILES = 256
_W2_TAIL = (128, 192, 64)
_V_SPLIT = 24
_LAST_ISSUE = 8

_SEM_K, _SEM_V, _SEM_WO, _SEM_WQ, _SEM_W1, _SEM_SMALL, _SEM_VX, _SEM_W2 = 0, 2, 4, 5, 6, 7, 11, 12
_N_SEMS = _SEM_W2 + 1 + len(_W2_TAIL)


def _spread(main, extra, phase):
    out, j = [], 0
    for i, item in enumerate(main):
        out.append(item)
        while j < len(extra) and (j + phase) / len(extra) <= (i + 1) / len(main):
            out.append(extra[j])
            j += 1
    return out + extra[j:]


def _halves(items):
    return items[:len(items) // 2], items[len(items) // 2:]


def _tile_groups(w):
    r, c = w.shape
    tiles = w.reshape(r // _SUB, _SUB, c // _LANES, _LANES).transpose(0, 2, 1, 3)
    return tiles.reshape(-1, _GROUP_TILES * _SUB, _LANES)


def _make_kernel(D, F, Sk, W):
    scale = _DH ** -0.5
    n_pairs = _HQ // 2
    pair_tiles = 2 * _DH // _LANES
    d_tiles = D // _LANES
    col0 = Sk - W
    tail_rows = sum(_W2_TAIL)
    tail0 = F - tail_rows
    nt_dims = (((1,), (1,)), ((), ()))
    group_rows = _GROUP_TILES * _SUB
    head_rows = _DH * d_tiles
    piece_rows = math.gcd(head_rows, group_rows)

    def body(x_hbm, k_hbm, v_hbm, wq_hbm, wo_hbm, w1_hbm, b1_hbm, w2_hbm, b2_hbm, gw_hbm,
             kbuf, vbuf, wqbuf, wobuf, w1buf, w2buf, xbuf, b1buf, b2buf, gwbuf, qbuf, pvbuf,
             obuf, sems):

        def tiles(src, dst, r0, c0, n_rows, n_cols, shape, sem):
            tr, tc = shape

            def maker(r, c):
                return lambda: pltpu.make_async_copy(
                    src.at[pl.ds(r0 + r, tr), pl.ds(c0 + c, tc)],
                    dst.at[pl.ds(r0 + r, tr), pl.ds(c, tc)], sems.at[sem])

            return [maker(r, c) for r in range(0, n_rows, tr) for c in range(0, n_cols, tc)]

        def tile_streams(src, dst, sem):
            def maker(t):
                rows = pl.ds(t * _SUB, _SUB)
                return lambda: pltpu.make_async_copy(
                    src.at[:, rows, :], dst.at[:, rows, :], sems.at[sem])

            return [maker(t) for t in range(_GROUP_TILES)]

        def block(src, dst, sem, riders=([], []), split=None):
            def slabs(sem):
                rows_a = _DH - _ROWS_B
                return (tiles(src, dst, _ROWS_B, col0, rows_a, W, (rows_a, _LANES), sem),
                        tiles(src, dst, 0, col0, _ROWS_B, W, (_ROWS_B, _LANES), sem))

            a, b = slabs(sem)
            if split is not None:
                a2, b2 = slabs(_SEM_VX)
                a, b = a[:split] + a2[split:], b[:split] + b2[split:]
            return _spread(a, riders[0], _PHASE_A), _spread(b, riders[1], _PHASE_B)

        def k_block(h, s, *args):
            return block(k_hbm.at[0, h], kbuf.at[s], _SEM_K + s, *args)

        def v_block(h, s, *args):
            return block(v_hbm.at[0, h], vbuf.at[s], _SEM_V + s, *args)

        w1_a, w1_b = _halves(tiles(w1_hbm, w1buf, 0, 0, D, F, (16, F), _SEM_W1))
        w2_a, w2_b = _halves(tiles(w2_hbm, w2buf, 0, 0, tail0, D, (32, D), _SEM_W2))
        mlp_a, mlp_b = w1_a + w2_a, w1_b + w2_b
        cuts = [round(i * len(mlp_a) / 4) for i in range(5)]
        riders = [(mlp_a[cuts[i]:cuts[i + 1]], mlp_b[cuts[i]:cuts[i + 1]]) for i in range(4)]
        no_riders = [([], [])] * 4
        w2_end, r0 = [], tail0
        for i, rows in enumerate(_W2_TAIL):
            w2_end += tiles(w2_hbm, w2buf, r0, 0, rows, D, (16, D), _SEM_W2 + 1 + i)
            r0 += rows

        def wait_full(buf, sem):
            pltpu.make_async_copy(buf, buf, sems.at[sem]).wait()

        def issue(a, b):
            for i in range(max(len(a), len(b))):
                if i < len(b):
                    b[i]().start(priority=1)
                if i < len(a):
                    a[i]().start(priority=0)

        small = [
            pltpu.make_async_copy(src, dst, sems.at[_SEM_SMALL + i])
            for i, (src, dst) in enumerate(
                ((x_hbm, xbuf), (gw_hbm, gwbuf), (b1_hbm, b1buf), (b2_hbm, b2buf)))
        ]

        def tiled_matvec(lhs, w_tiles, cols):
            rows = w_tiles.shape[0] * _SUB
            return jnp.concatenate(
                [jnp.dot(lhs, w_tiles[:, c].reshape(rows, _LANES),
                         preferred_element_type=_F32) for c in cols], axis=1)

        k0a, k0b = k_block(0, 0)
        v0a, v0b = v_block(0, 0)
        pro_b = tile_streams(wo_hbm, wobuf, _SEM_WO) + k0b + v0b[:_LEAD]
        issue([], pro_b[:_LEAD])
        for cp in small:
            cp.start()
        issue(tile_streams(wq_hbm, wqbuf, _SEM_WQ) + k0a, pro_b[_LEAD:])

        small[0].wait()
        small[1].wait()
        wait_full(wqbuf, _SEM_WQ)
        x = xbuf[0].astype(_F32)
        x8 = jnp.broadcast_to(x, (8, D)).astype(_BF16)
        gate = jax.nn.sigmoid(jnp.sum(
            x * gwbuf[...].reshape(1, D).astype(_F32), axis=-1, keepdims=True))

        pro_b = v0b[_LEAD:] + k_block(1, 1, riders[0])[1][:_LEAD]
        separators = [small[2].wait, small[3].wait, lambda: wait_full(wobuf, _SEM_WO)]
        n_parts = len(separators) + 1
        for part in range(n_parts):
            if part > 0:
                separators[part - 1]()
            wq_tiles = wqbuf[...].reshape(D // _SUB, n_pairs * pair_tiles, _SUB, _LANES)
            for p in range(part * n_pairs // n_parts, (part + 1) * n_pairs // n_parts):
                qbuf[p] = tiled_matvec(x8, wq_tiles, range(p * pair_tiles, (p + 1) * pair_tiles))
            sl = slice(part * len(v0a) // n_parts, (part + 1) * len(v0a) // n_parts)
            issue(v0a[sl], pro_b[sl])

        def scores(q, s):
            wait_full(kbuf.at[s], _SEM_K + s)
            sc = jnp.dot(q, kbuf[s], preferred_element_type=_F32) * scale
            e = jnp.exp(sc - jnp.max(sc, axis=-1, keepdims=True))
            return e.astype(_BF16), jnp.sum(e, axis=-1, keepdims=True)

        def out_proj(o, l, h):
            pieces = []
            for r in range(0, head_rows, piece_rows):
                r = h * head_rows + r
                if isinstance(r, int):
                    g, off = divmod(r, group_rows)
                else:
                    g = jax.lax.div(r, group_rows)
                    off = pl.multiple_of(jax.lax.rem(r, group_rows), piece_rows)
                pieces.append(wobuf[g, pl.ds(off, piece_rows), :])
            wo_h = jnp.concatenate(pieces, axis=0).reshape(_DH // _SUB, d_tiles, _SUB, _LANES)
            return tiled_matvec((o / l).astype(_BF16), wo_h, range(d_tiles))

        def project(e, l, s, h):
            wait_full(vbuf.at[s], _SEM_V + s)
            o = jax.lax.dot_general(e, vbuf[s], nt_dims, preferred_element_type=_F32)
            return out_proj(o, l, h)

        st = {}

        def pair_step(p, acc, first=False, last=False):
            h = 2 * p
            extra = riders if first else no_riders
            k1a, k1b = k_block(h + 1, 1, extra[0])
            v1a, v1b = v_block(h + 1, 1, extra[1], _V_SPLIT if last else None)

            issue(k1a, k1b[_LEAD:] + v1b[:_LEAD])
            if last:
                wait_full(w1buf, _SEM_W1)
                hid = jnp.dot(x8, w1buf[...], preferred_element_type=_F32)
                hid = hid + b1buf[...].reshape(1, F).astype(_F32)
                hid = jax.nn.gelu(hid, approximate=True).astype(_BF16)
                tail = hid[0:1, tail0:].astype(_F32) * (1.0 - gate)
                st['hcol'] = jnp.broadcast_to(tail, (_LANES, tail_rows)).T
            q2 = qbuf[p].astype(_BF16)
            e, l = scores(q2[:, :_DH], 0)

            if not last:
                k2a, k2b = k_block(h + 2, 0, extra[2])
                v2a, v2b = v_block(h + 2, 0, extra[3])
                issue(v1a, v1b[_LEAD:] + k2b[:_LEAD])
                acc = acc + project(e, l, 0, h)
                issue(k2a, k2b[_LEAD:] + v2b[:_LEAD])
                e, l = scores(q2[:, _DH:], 1)
                issue(v2a, v2b[_LEAD:] + k_block(h + 3, 1)[1][:_LEAD])
                return acc + project(e, l, 1, h + 1)

            b_end = v1b[_LEAD:] + w2_end
            issue(v1a[:_LAST_ISSUE], b_end[:_LAST_ISSUE])
            acc = acc + project(e, l, 0, h)
            wait_full(w2buf.at[pl.ds(0, tail0)], _SEM_W2)
            st['mlp'] = b2buf[...].reshape(1, D).astype(_F32) + jnp.dot(
                hid[:, :tail0], w2buf[0:tail0, :], preferred_element_type=_F32)
            issue(v1a[_LAST_ISSUE:], b_end[_LAST_ISSUE:])
            e, l = scores(q2[:, _DH:], 1)
            cs = _V_SPLIT * _LANES
            wait_full(vbuf.at[1, :, pl.ds(0, cs)], _SEM_V + 1)
            pvbuf[...] = jax.lax.dot_general(e[:, :cs], vbuf[1, :, :cs], nt_dims,
                                             preferred_element_type=_F32)
            wait_full(vbuf.at[1, :, pl.ds(cs, W - cs)], _SEM_VX)
            o = pvbuf[...] + jax.lax.dot_general(e[:, cs:], vbuf[1, :, cs:], nt_dims,
                                                 preferred_element_type=_F32)
            return acc + out_proj(o, l, h + 1)

        acc = pair_step(0, jnp.zeros((8, D), _F32), first=True)
        acc = jax.lax.fori_loop(1, n_pairs - 1, pair_step, acc)
        att = pair_step(n_pairs - 1, acc, last=True)

        base = gate * att + (1.0 - gate) * st['mlp']
        row = jax.lax.broadcasted_iota(jnp.int32, (8, D), 0)
        part = jnp.where(row == 0, base, 0.0)
        r0 = tail0
        for i, rows in enumerate(_W2_TAIL):
            wait_full(w2buf.at[pl.ds(r0, rows)], _SEM_W2 + 1 + i)
            hcol = st['hcol'][r0 - tail0:r0 - tail0 + rows]
            sums = []
            for c in range(d_tiles):
                w = w2buf[r0:r0 + rows, c * _LANES:(c + 1) * _LANES].astype(_F32)
                sums.append(jnp.sum((w * hcol).reshape(rows // 8, 8, _LANES), axis=0))
            part = part + jnp.concatenate(sums, axis=1)
            r0 += rows
        obuf[0] = jnp.sum(part, axis=0, keepdims=True).astype(obuf.dtype)

    def kernel(*refs):
        ins, o_hbm, scratch, out_sem = refs[:10], refs[10], refs[11:-1], refs[-1]
        out_copy = pltpu.make_async_copy(scratch[-1], o_hbm, out_sem.at[0])

        def scoped(sems):
            body(*ins, *scratch, sems)
            out_copy.start()

        pl.run_scoped(scoped, pltpu.SemaphoreType.DMA((_N_SEMS,)))
        out_copy.wait()

    return kernel


@jax.jit
def pallas_gated_mix__sliding_block_cached__dense_activation_gelu__decode_kernel(
    A_x: jax.Array,
    A_k_cache: jax.Array,
    A_v_cache: jax.Array,
    A_wq: jax.Array,
    A_wo: jax.Array,
    B_x: jax.Array,
    B_w1: jax.Array,
    B_b1: jax.Array,
    B_w2: jax.Array,
    B_b2: jax.Array,
    gate_w: jax.Array,
):
    del B_x
    B, Sq, D = A_x.shape
    _, Hkv, Sk, Dh = A_k_cache.shape
    F = B_w1.shape[1]
    assert (B, Sq, Hkv, Dh) == (1, 1, _HQ, _DH)
    W = min(4096, max(256, Sk // 4))
    assert W // _LANES > max(_LEAD, _V_SPLIT)

    kt = jnp.swapaxes(A_k_cache, 2, 3)
    vt = jnp.swapaxes(A_v_cache, 2, 3)
    wq_t = _tile_groups(A_wq)
    wo_t = _tile_groups(A_wo)

    return pl.pallas_call(
        _make_kernel(D, F, Sk, W),
        out_shape=jax.ShapeDtypeStruct((B, Sq, D), A_x.dtype),
        in_specs=[pl.BlockSpec(memory_space=pl.ANY)] * 10,
        out_specs=pl.BlockSpec(memory_space=pl.ANY),
        scratch_shapes=[
            pltpu.VMEM((2, _DH, W), _BF16),
            pltpu.VMEM((2, _DH, W), _BF16),
            pltpu.VMEM(wq_t.shape, _BF16),
            pltpu.VMEM(wo_t.shape, _BF16),
            pltpu.VMEM((D, F), _BF16),
            pltpu.VMEM((F, D), _BF16),
            pltpu.VMEM((1, 1, D), _BF16),
            pltpu.VMEM((F,), _BF16),
            pltpu.VMEM((D,), _BF16),
            pltpu.VMEM((D,), _BF16),
            pltpu.VMEM((_HQ // 2, 8, 2 * _DH), _F32),
            pltpu.VMEM((8, _DH), _F32),
            pltpu.VMEM((1, 1, D), _BF16),
            pltpu.SemaphoreType.DMA((1,)),
        ],
        compiler_params=pltpu.CompilerParams(vmem_limit_bytes=64 * 1024 * 1024),
    )(A_x, kt, vt, wq_t, wo_t, B_w1, B_b1, B_w2, B_b2, gate_w)
```

```python
import math

import jax
import jax.numpy as jnp
import jax.experimental.pallas as pl
import jax.experimental.pallas.tpu as pltpu

_F32 = jnp.float32
_BF16 = jnp.bfloat16
_LANES = 128
_SUB = 8

_HQ = 32
_DH = 192

_LEAD = 25
_ROWS_B = 128
_PHASE_A, _PHASE_B = 0.25, 0.75
_GROUP_TILES = 256
_W2_TAIL = (128, 192, 64)
_V_SPLIT = 24
_LAST_ISSUE = 8

_SEM_K, _SEM_V, _SEM_WO, _SEM_WQ, _SEM_W1, _SEM_SMALL = 0, 2, 4, 5, 6, 7
_SEM_VX, _SEM_OUT, _SEM_W2 = 11, 12, 13
_N_SEMS = _SEM_W2 + 1 + len(_W2_TAIL)


def _spread(main, extra, phase):
    out, j = [], 0
    for i, item in enumerate(main):
        out.append(item)
        while j < len(extra) and (j + phase) / len(extra) <= (i + 1) / len(main):
            out.append(extra[j])
            j += 1
    return out + extra[j:]


def _halves(items):
    return items[:len(items) // 2], items[len(items) // 2:]


def _tile_groups(w):
    r, c = w.shape
    tiles = w.reshape(r // _SUB, _SUB, c // _LANES, _LANES).transpose(0, 2, 1, 3)
    return tiles.reshape(-1, _GROUP_TILES * _SUB, _LANES)


def _make_kernel(D, F, Sk, W):
    scale = _DH ** -0.5
    n_pairs = _HQ // 2
    pair_tiles = 2 * _DH // _LANES
    d_tiles = D // _LANES
    col0 = Sk - W
    tail_rows = sum(_W2_TAIL)
    tail0 = F - tail_rows
    nt_dims = (((1,), (1,)), ((), ()))
    group_rows = _GROUP_TILES * _SUB
    head_rows = _DH * d_tiles
    piece_rows = math.gcd(head_rows, group_rows)

    def body(x_hbm, k_hbm, v_hbm, wq_hbm, wo_hbm, w1_hbm, b1_hbm, w2_hbm, b2_hbm, gw_hbm,
             o_hbm, kbuf, vbuf, wqbuf, wobuf, w1buf, w2buf, xbuf, b1buf, b2buf, gwbuf, qbuf,
             pvbuf, obuf, sems):

        def tiles(src, dst, r0, c0, n_rows, n_cols, shape, sem):
            tr, tc = shape

            def maker(r, c):
                return lambda: pltpu.make_async_copy(
                    src.at[pl.ds(r0 + r, tr), pl.ds(c0 + c, tc)],
                    dst.at[pl.ds(r0 + r, tr), pl.ds(c, tc)], sems.at[sem])

            return [maker(r, c) for r in range(0, n_rows, tr) for c in range(0, n_cols, tc)]

        def tile_streams(src, dst, sem):
            def maker(t):
                rows = pl.ds(t * _SUB, _SUB)
                return lambda: pltpu.make_async_copy(
                    src.at[:, rows, :], dst.at[:, rows, :], sems.at[sem])

            return [maker(t) for t in range(_GROUP_TILES)]

        def block(src, dst, sem, riders=([], []), split=None):
            def slabs(sem):
                rows_a = _DH - _ROWS_B
                return (tiles(src, dst, _ROWS_B, col0, rows_a, W, (rows_a, _LANES), sem),
                        tiles(src, dst, 0, col0, _ROWS_B, W, (_ROWS_B, _LANES), sem))

            a, b = slabs(sem)
            if split is not None:
                a2, b2 = slabs(_SEM_VX)
                a, b = a[:split] + a2[split:], b[:split] + b2[split:]
            return _spread(a, riders[0], _PHASE_A), _spread(b, riders[1], _PHASE_B)

        def k_block(h, s, *args):
            return block(k_hbm.at[0, h], kbuf.at[s], _SEM_K + s, *args)

        def v_block(h, s, *args):
            return block(v_hbm.at[0, h], vbuf.at[s], _SEM_V + s, *args)

        w1_a, w1_b = _halves(tiles(w1_hbm, w1buf, 0, 0, D, F, (16, F), _SEM_W1))
        w2_a, w2_b = _halves(tiles(w2_hbm, w2buf, 0, 0, tail0, D, (32, D), _SEM_W2))
        mlp_a, mlp_b = w1_a + w2_a, w1_b + w2_b
        cuts = [round(i * len(mlp_a) / 4) for i in range(5)]
        riders = [(mlp_a[cuts[i]:cuts[i + 1]], mlp_b[cuts[i]:cuts[i + 1]]) for i in range(4)]
        no_riders = [([], [])] * 4
        w2_end, r0 = [], tail0
        for i, rows in enumerate(_W2_TAIL):
            w2_end += tiles(w2_hbm, w2buf, r0, 0, rows, D, (16, D), _SEM_W2 + 1 + i)
            r0 += rows

        def wait_full(buf, sem):
            pltpu.make_async_copy(buf, buf, sems.at[sem]).wait()

        def issue(a, b):
            for i in range(max(len(a), len(b))):
                if i < len(b):
                    b[i]().start(priority=1)
                if i < len(a):
                    a[i]().start(priority=0)

        small = [
            pltpu.make_async_copy(src, dst, sems.at[_SEM_SMALL + i])
            for i, (src, dst) in enumerate(
                ((x_hbm, xbuf), (gw_hbm, gwbuf), (b1_hbm, b1buf), (b2_hbm, b2buf)))
        ]

        def tiled_matvec(lhs, w_tiles, cols):
            rows = w_tiles.shape[0] * _SUB
            return jnp.concatenate(
                [jnp.dot(lhs, w_tiles[:, c].reshape(rows, _LANES),
                         preferred_element_type=_F32) for c in cols], axis=1)

        k0a, k0b = k_block(0, 0)
        v0a, v0b = v_block(0, 0)
        pro_b = tile_streams(wo_hbm, wobuf, _SEM_WO) + k0b + v0b[:_LEAD]
        issue([], pro_b[:_LEAD])
        for cp in small:
            cp.start()
        issue(tile_streams(wq_hbm, wqbuf, _SEM_WQ) + k0a, pro_b[_LEAD:])

        small[0].wait()
        small[1].wait()
        wait_full(wqbuf, _SEM_WQ)
        x = xbuf[0].astype(_F32)
        x8 = jnp.broadcast_to(x, (8, D)).astype(_BF16)
        gate = jax.nn.sigmoid(jnp.sum(
            x * gwbuf[...].reshape(1, D).astype(_F32), axis=-1, keepdims=True))

        pro_b = v0b[_LEAD:] + k_block(1, 1, riders[0])[1][:_LEAD]
        separators = [small[2].wait, small[3].wait, lambda: wait_full(wobuf, _SEM_WO)]
        n_parts = len(separators) + 1
        for part in range(n_parts):
            if part > 0:
                separators[part - 1]()
            wq_tiles = wqbuf[...].reshape(D // _SUB, n_pairs * pair_tiles, _SUB, _LANES)
            for p in range(part * n_pairs // n_parts, (part + 1) * n_pairs // n_parts):
                qbuf[p] = tiled_matvec(x8, wq_tiles, range(p * pair_tiles, (p + 1) * pair_tiles))
            sl = slice(part * len(v0a) // n_parts, (part + 1) * len(v0a) // n_parts)
            issue(v0a[sl], pro_b[sl])

        def scores(q, s):
            wait_full(kbuf.at[s], _SEM_K + s)
            sc = jnp.dot(q, kbuf[s], preferred_element_type=_F32) * scale
            e = jnp.exp(sc - jnp.max(sc, axis=-1, keepdims=True))
            return e.astype(_BF16), jnp.sum(e, axis=-1, keepdims=True)

        def out_proj(o, l, h):
            pieces = []
            for r in range(0, head_rows, piece_rows):
                r = h * head_rows + r
                if isinstance(r, int):
                    g, off = divmod(r, group_rows)
                else:
                    g = jax.lax.div(r, group_rows)
                    off = pl.multiple_of(jax.lax.rem(r, group_rows), piece_rows)
                pieces.append(wobuf[g, pl.ds(off, piece_rows), :])
            wo_h = jnp.concatenate(pieces, axis=0).reshape(_DH // _SUB, d_tiles, _SUB, _LANES)
            return tiled_matvec((o / l).astype(_BF16), wo_h, range(d_tiles))

        def project(e, l, s, h):
            wait_full(vbuf.at[s], _SEM_V + s)
            o = jax.lax.dot_general(e, vbuf[s], nt_dims, preferred_element_type=_F32)
            return out_proj(o, l, h)

        st = {}

        def pair_step(p, acc, first=False, last=False):
            h = 2 * p
            extra = riders if first else no_riders
            k1a, k1b = k_block(h + 1, 1, extra[0])
            v1a, v1b = v_block(h + 1, 1, extra[1], _V_SPLIT if last else None)

            issue(k1a, k1b[_LEAD:] + v1b[:_LEAD])
            if last:
                wait_full(w1buf, _SEM_W1)
                hid = jnp.dot(x8, w1buf[...], preferred_element_type=_F32)
                hid = hid + b1buf[...].reshape(1, F).astype(_F32)
                hid = jax.nn.gelu(hid, approximate=True).astype(_BF16)
                tail = hid[0:1, tail0:].astype(_F32) * (1.0 - gate)
                st['hcol'] = jnp.broadcast_to(tail, (_LANES, tail_rows)).T
            q2 = qbuf[p].astype(_BF16)
            e, l = scores(q2[:, :_DH], 0)

            if not last:
                k2a, k2b = k_block(h + 2, 0, extra[2])
                v2a, v2b = v_block(h + 2, 0, extra[3])
                issue(v1a, v1b[_LEAD:] + k2b[:_LEAD])
                acc = acc + project(e, l, 0, h)
                issue(k2a, k2b[_LEAD:] + v2b[:_LEAD])
                e, l = scores(q2[:, _DH:], 1)
                issue(v2a, v2b[_LEAD:] + k_block(h + 3, 1)[1][:_LEAD])
                return acc + project(e, l, 1, h + 1)

            b_end = v1b[_LEAD:] + w2_end
            issue(v1a[:_LAST_ISSUE], b_end[:_LAST_ISSUE])
            acc = acc + project(e, l, 0, h)
            wait_full(w2buf.at[pl.ds(0, tail0)], _SEM_W2)
            st['mlp'] = b2buf[...].reshape(1, D).astype(_F32) + jnp.dot(
                hid[:, :tail0], w2buf[0:tail0, :], preferred_element_type=_F32)
            issue(v1a[_LAST_ISSUE:], b_end[_LAST_ISSUE:])
            e, l = scores(q2[:, _DH:], 1)
            cs = _V_SPLIT * _LANES
            wait_full(vbuf.at[1, :, pl.ds(0, cs)], _SEM_V + 1)
            pvbuf[...] = jax.lax.dot_general(e[:, :cs], vbuf[1, :, :cs], nt_dims,
                                             preferred_element_type=_F32)
            wait_full(vbuf.at[1, :, pl.ds(cs, W - cs)], _SEM_VX)
            o = pvbuf[...] + jax.lax.dot_general(e[:, cs:], vbuf[1, :, cs:], nt_dims,
                                                 preferred_element_type=_F32)
            return acc + out_proj(o, l, h + 1)

        acc = pair_step(0, jnp.zeros((8, D), _F32), first=True)
        acc = jax.lax.fori_loop(1, n_pairs - 1, pair_step, acc)
        att = pair_step(n_pairs - 1, acc, last=True)

        base = gate * att + (1.0 - gate) * st['mlp']
        row = jax.lax.broadcasted_iota(jnp.int32, (8, D), 0)
        part = jnp.where(row == 0, base, 0.0)
        r0 = tail0
        for i, rows in enumerate(_W2_TAIL):
            wait_full(w2buf.at[pl.ds(r0, rows)], _SEM_W2 + 1 + i)
            hcol = st['hcol'][r0 - tail0:r0 - tail0 + rows]
            sums = []
            for c in range(d_tiles):
                w = w2buf[r0:r0 + rows, c * _LANES:(c + 1) * _LANES].astype(_F32)
                sums.append(jnp.sum((w * hcol).reshape(rows // 8, 8, _LANES), axis=0))
            part = part + jnp.concatenate(sums, axis=1)
            r0 += rows
        obuf[0] = jnp.sum(part, axis=0, keepdims=True).astype(obuf.dtype)
        out_copy = pltpu.make_async_copy(obuf, o_hbm, sems.at[_SEM_OUT])
        out_copy.start()
        out_copy.wait()

    def kernel(*refs):
        pl.run_scoped(lambda sems: body(*refs, sems), pltpu.SemaphoreType.DMA((_N_SEMS,)))

    return kernel


@jax.jit
def pallas_gated_mix__sliding_block_cached__dense_activation_gelu__decode_kernel(
    A_x: jax.Array,
    A_k_cache: jax.Array,
    A_v_cache: jax.Array,
    A_wq: jax.Array,
    A_wo: jax.Array,
    B_x: jax.Array,
    B_w1: jax.Array,
    B_b1: jax.Array,
    B_w2: jax.Array,
    B_b2: jax.Array,
    gate_w: jax.Array,
):
    del B_x
    B, Sq, D = A_x.shape
    _, Hkv, Sk, Dh = A_k_cache.shape
    F = B_w1.shape[1]
    assert (B, Sq, Hkv, Dh) == (1, 1, _HQ, _DH)
    W = min(4096, max(256, Sk // 4))
    assert W // _LANES > max(_LEAD, _V_SPLIT)

    kt = jnp.swapaxes(A_k_cache, 2, 3)
    vt = jnp.swapaxes(A_v_cache, 2, 3)
    wq_t = _tile_groups(A_wq)
    wo_t = _tile_groups(A_wo)

    return pl.pallas_call(
        _make_kernel(D, F, Sk, W),
        out_shape=jax.ShapeDtypeStruct((B, Sq, D), A_x.dtype),
        in_specs=[pl.BlockSpec(memory_space=pl.ANY)] * 10,
        out_specs=pl.BlockSpec(memory_space=pl.ANY),
        scratch_shapes=[
            pltpu.VMEM((2, _DH, W), _BF16),
            pltpu.VMEM((2, _DH, W), _BF16),
            pltpu.VMEM(wq_t.shape, _BF16),
            pltpu.VMEM(wo_t.shape, _BF16),
            pltpu.VMEM((D, F), _BF16),
            pltpu.VMEM((F, D), _BF16),
            pltpu.VMEM((1, 1, D), _BF16),
            pltpu.VMEM((F,), _BF16),
            pltpu.VMEM((D,), _BF16),
            pltpu.VMEM((D,), _BF16),
            pltpu.VMEM((_HQ // 2, 8, 2 * _DH), _F32),
            pltpu.VMEM((8, _DH), _F32),
            pltpu.VMEM((1, 1, D), _BF16),
        ],
        compiler_params=pltpu.CompilerParams(vmem_limit_bytes=64 * 1024 * 1024),
    )(A_x, kt, vt, wq_t, wo_t, B_w1, B_b1, B_w2, B_b2, gate_w)
```

```python
import math

import jax
import jax.numpy as jnp
import jax.experimental.pallas as pl
import jax.experimental.pallas.tpu as pltpu

_F32 = jnp.float32
_BF16 = jnp.bfloat16
_LANES = 128
_SUB = 8

_HQ = 32
_DH = 192

_LEAD = 25
_ROWS_B = 128
_PHASE_A, _PHASE_B = 0.25, 0.75
_GROUP_TILES = 256
_GROUPS_A = 4
_W2_TAIL = (128, 192, 64)
_V_SPLIT = 24
_LAST_ISSUE = 8

_SEM_K, _SEM_V, _SEM_WO, _SEM_WQ, _SEM_W1, _SEM_SMALL = 0, 2, 4, 5, 6, 7
_SEM_VX, _SEM_OUT, _SEM_W2 = 11, 12, 13
_N_SEMS = _SEM_W2 + 1 + len(_W2_TAIL)


def _spread(main, extra, phase):
    out, j = [], 0
    for i, item in enumerate(main):
        out.append(item)
        while j < len(extra) and (j + phase) / len(extra) <= (i + 1) / len(main):
            out.append(extra[j])
            j += 1
    return out + extra[j:]


def _halves(items):
    return items[:len(items) // 2], items[len(items) // 2:]


def _tile_groups(w):
    r, c = w.shape
    tiles = w.reshape(r // _SUB, _SUB, c // _LANES, _LANES).transpose(0, 2, 1, 3)
    return tiles.reshape(-1, _GROUP_TILES * _SUB, _LANES)


def _make_kernel(D, F, Sk, W):
    scale = _DH ** -0.5
    n_pairs = _HQ // 2
    pair_tiles = 2 * _DH // _LANES
    d_tiles = D // _LANES
    col0 = Sk - W
    tail_rows = sum(_W2_TAIL)
    tail0 = F - tail_rows
    nt_dims = (((1,), (1,)), ((), ()))
    group_rows = _GROUP_TILES * _SUB
    head_rows = _DH * d_tiles
    piece_rows = math.gcd(head_rows, group_rows)

    def body(x_hbm, k_hbm, v_hbm, wq_hbm, wo_hbm, w1_hbm, b1_hbm, w2_hbm, b2_hbm, gw_hbm,
             o_hbm, kbuf, vbuf, wqbuf, wobuf, w1buf, w2buf, xbuf, b1buf, b2buf, gwbuf, qbuf,
             pvbuf, obuf, sems):

        def tiles(src, dst, r0, c0, n_rows, n_cols, shape, sem):
            tr, tc = shape

            def maker(r, c):
                return lambda: pltpu.make_async_copy(
                    src.at[pl.ds(r0 + r, tr), pl.ds(c0 + c, tc)],
                    dst.at[pl.ds(r0 + r, tr), pl.ds(c, tc)], sems.at[sem])

            return [maker(r, c) for r in range(0, n_rows, tr) for c in range(0, n_cols, tc)]

        def tile_streams(src, dst, sem):
            groups_b = src.shape[0] - _GROUPS_A

            def maker(groups, t):
                rows = pl.ds(t * _SUB, _SUB)
                return lambda: pltpu.make_async_copy(
                    src.at[groups, rows, :], dst.at[groups, rows, :], sems.at[sem])

            return ([maker(pl.ds(groups_b, _GROUPS_A), t) for t in range(_GROUP_TILES)],
                    [maker(pl.ds(0, groups_b), t) for t in range(_GROUP_TILES)])

        def block(src, dst, sem, riders=([], []), split=None):
            def slabs(sem):
                rows_a = _DH - _ROWS_B
                return (tiles(src, dst, _ROWS_B, col0, rows_a, W, (rows_a, _LANES), sem),
                        tiles(src, dst, 0, col0, _ROWS_B, W, (_ROWS_B, _LANES), sem))

            a, b = slabs(sem)
            if split is not None:
                a2, b2 = slabs(_SEM_VX)
                a, b = a[:split] + a2[split:], b[:split] + b2[split:]
            return _spread(a, riders[0], _PHASE_A), _spread(b, riders[1], _PHASE_B)

        def k_block(h, s, *args):
            return block(k_hbm.at[0, h], kbuf.at[s], _SEM_K + s, *args)

        def v_block(h, s, *args):
            return block(v_hbm.at[0, h], vbuf.at[s], _SEM_V + s, *args)

        w1_a, w1_b = _halves(tiles(w1_hbm, w1buf, 0, 0, D, F, (16, F), _SEM_W1))
        w2_a, w2_b = _halves(tiles(w2_hbm, w2buf, 0, 0, tail0, D, (32, D), _SEM_W2))
        mlp_a, mlp_b = w1_a + w2_a, w1_b + w2_b
        cuts = [round(i * len(mlp_a) / 4) for i in range(5)]
        riders = [(mlp_a[cuts[i]:cuts[i + 1]], mlp_b[cuts[i]:cuts[i + 1]]) for i in range(4)]
        no_riders = [([], [])] * 4
        w2_end, r0 = [], tail0
        for i, rows in enumerate(_W2_TAIL):
            w2_end += tiles(w2_hbm, w2buf, r0, 0, rows, D, (16, D), _SEM_W2 + 1 + i)
            r0 += rows

        def wait_full(buf, sem):
            pltpu.make_async_copy(buf, buf, sems.at[sem]).wait()

        def issue(a, b):
            for i in range(max(len(a), len(b))):
                if i < len(b):
                    b[i]().start(priority=1)
                if i < len(a):
                    a[i]().start(priority=0)

        small = [
            pltpu.make_async_copy(src, dst, sems.at[_SEM_SMALL + i])
            for i, (src, dst) in enumerate(
                ((x_hbm, xbuf), (gw_hbm, gwbuf), (b1_hbm, b1buf), (b2_hbm, b2buf)))
        ]

        def tiled_matvec(lhs, w_tiles, cols):
            rows = w_tiles.shape[0] * _SUB
            return jnp.concatenate(
                [jnp.dot(lhs, w_tiles[:, c].reshape(rows, _LANES),
                         preferred_element_type=_F32) for c in cols], axis=1)

        k0a, k0b = k_block(0, 0)
        v0a, v0b = v_block(0, 0)
        wq_a, wq_b = tile_streams(wq_hbm, wqbuf, _SEM_WQ)
        wo_a, wo_b = tile_streams(wo_hbm, wobuf, _SEM_WO)
        pro_b = wq_b + wo_b + k0b + v0b[:_LEAD]
        issue([], pro_b[:_LEAD])
        for cp in small:
            cp.start()
        issue(wq_a + wo_a + k0a, pro_b[_LEAD:])

        small[0].wait()
        small[1].wait()
        wait_full(wqbuf, _SEM_WQ)
        x = xbuf[0].astype(_F32)
        x8 = jnp.broadcast_to(x, (8, D)).astype(_BF16)
        gate = jax.nn.sigmoid(jnp.sum(
            x * gwbuf[...].reshape(1, D).astype(_F32), axis=-1, keepdims=True))

        pro_b = v0b[_LEAD:] + k_block(1, 1, riders[0])[1][:_LEAD]
        separators = [small[2].wait, small[3].wait, lambda: wait_full(wobuf, _SEM_WO)]
        n_parts = len(separators) + 1
        for part in range(n_parts):
            if part > 0:
                separators[part - 1]()
            wq_tiles = wqbuf[...].reshape(D // _SUB, n_pairs * pair_tiles, _SUB, _LANES)
            for p in range(part * n_pairs // n_parts, (part + 1) * n_pairs // n_parts):
                qbuf[p] = tiled_matvec(x8, wq_tiles, range(p * pair_tiles, (p + 1) * pair_tiles))
            sl = slice(part * len(v0a) // n_parts, (part + 1) * len(v0a) // n_parts)
            issue(v0a[sl], pro_b[sl])

        def scores(q, s):
            wait_full(kbuf.at[s], _SEM_K + s)
            sc = jnp.dot(q, kbuf[s], preferred_element_type=_F32) * scale
            e = jnp.exp(sc - jnp.max(sc, axis=-1, keepdims=True))
            return e.astype(_BF16), jnp.sum(e, axis=-1, keepdims=True)

        def out_proj(o, l, h):
            pieces = []
            for r in range(0, head_rows, piece_rows):
                r = h * head_rows + r
                if isinstance(r, int):
                    g, off = divmod(r, group_rows)
                else:
                    g = jax.lax.div(r, group_rows)
                    off = pl.multiple_of(jax.lax.rem(r, group_rows), piece_rows)
                pieces.append(wobuf[g, pl.ds(off, piece_rows), :])
            wo_h = jnp.concatenate(pieces, axis=0).reshape(_DH // _SUB, d_tiles, _SUB, _LANES)
            return tiled_matvec((o / l).astype(_BF16), wo_h, range(d_tiles))

        def project(e, l, s, h):
            wait_full(vbuf.at[s], _SEM_V + s)
            o = jax.lax.dot_general(e, vbuf[s], nt_dims, preferred_element_type=_F32)
            return out_proj(o, l, h)

        st = {}

        def pair_step(p, acc, first=False, last=False):
            h = 2 * p
            extra = riders if first else no_riders
            k1a, k1b = k_block(h + 1, 1, extra[0])
            v1a, v1b = v_block(h + 1, 1, extra[1], _V_SPLIT if last else None)

            issue(k1a, k1b[_LEAD:] + v1b[:_LEAD])
            if last:
                wait_full(w1buf, _SEM_W1)
                hid = jnp.dot(x8, w1buf[...], preferred_element_type=_F32)
                hid = hid + b1buf[...].reshape(1, F).astype(_F32)
                hid = jax.nn.gelu(hid, approximate=True).astype(_BF16)
                tail = hid[0:1, tail0:].astype(_F32) * (1.0 - gate)
                st['hcol'] = jnp.broadcast_to(tail, (_LANES, tail_rows)).T
            q2 = qbuf[p].astype(_BF16)
            e, l = scores(q2[:, :_DH], 0)

            if not last:
                k2a, k2b = k_block(h + 2, 0, extra[2])
                v2a, v2b = v_block(h + 2, 0, extra[3])
                issue(v1a, v1b[_LEAD:] + k2b[:_LEAD])
                acc = acc + project(e, l, 0, h)
                issue(k2a, k2b[_LEAD:] + v2b[:_LEAD])
                e, l = scores(q2[:, _DH:], 1)
                issue(v2a, v2b[_LEAD:] + k_block(h + 3, 1)[1][:_LEAD])
                return acc + project(e, l, 1, h + 1)

            b_end = v1b[_LEAD:] + w2_end
            issue(v1a[:_LAST_ISSUE], b_end[:_LAST_ISSUE])
            acc = acc + project(e, l, 0, h)
            wait_full(w2buf.at[pl.ds(0, tail0)], _SEM_W2)
            st['mlp'] = b2buf[...].reshape(1, D).astype(_F32) + jnp.dot(
                hid[:, :tail0], w2buf[0:tail0, :], preferred_element_type=_F32)
            issue(v1a[_LAST_ISSUE:], b_end[_LAST_ISSUE:])
            e, l = scores(q2[:, _DH:], 1)
            cs = _V_SPLIT * _LANES
            wait_full(vbuf.at[1, :, pl.ds(0, cs)], _SEM_V + 1)
            pvbuf[...] = jax.lax.dot_general(e[:, :cs], vbuf[1, :, :cs], nt_dims,
                                             preferred_element_type=_F32)
            wait_full(vbuf.at[1, :, pl.ds(cs, W - cs)], _SEM_VX)
            o = pvbuf[...] + jax.lax.dot_general(e[:, cs:], vbuf[1, :, cs:], nt_dims,
                                                 preferred_element_type=_F32)
            return acc + out_proj(o, l, h + 1)

        acc = pair_step(0, jnp.zeros((8, D), _F32), first=True)
        acc = jax.lax.fori_loop(1, n_pairs - 1, pair_step, acc)
        att = pair_step(n_pairs - 1, acc, last=True)

        base = gate * att + (1.0 - gate) * st['mlp']
        row = jax.lax.broadcasted_iota(jnp.int32, (8, D), 0)
        part = jnp.where(row == 0, base, 0.0)
        r0 = tail0
        for i, rows in enumerate(_W2_TAIL):
            wait_full(w2buf.at[pl.ds(r0, rows)], _SEM_W2 + 1 + i)
            hcol = st['hcol'][r0 - tail0:r0 - tail0 + rows]
            sums = []
            for c in range(d_tiles):
                w = w2buf[r0:r0 + rows, c * _LANES:(c + 1) * _LANES].astype(_F32)
                sums.append(jnp.sum((w * hcol).reshape(rows // 8, 8, _LANES), axis=0))
            part = part + jnp.concatenate(sums, axis=1)
            r0 += rows
        obuf[0] = jnp.sum(part, axis=0, keepdims=True).astype(obuf.dtype)
        out_copy = pltpu.make_async_copy(obuf, o_hbm, sems.at[_SEM_OUT])
        out_copy.start()
        out_copy.wait()

    def kernel(*refs):
        pl.run_scoped(lambda sems: body(*refs, sems), pltpu.SemaphoreType.DMA((_N_SEMS,)))

    return kernel


@jax.jit
def pallas_gated_mix__sliding_block_cached__dense_activation_gelu__decode_kernel(
    A_x: jax.Array,
    A_k_cache: jax.Array,
    A_v_cache: jax.Array,
    A_wq: jax.Array,
    A_wo: jax.Array,
    B_x: jax.Array,
    B_w1: jax.Array,
    B_b1: jax.Array,
    B_w2: jax.Array,
    B_b2: jax.Array,
    gate_w: jax.Array,
):
    del B_x
    B, Sq, D = A_x.shape
    _, Hkv, Sk, Dh = A_k_cache.shape
    F = B_w1.shape[1]
    assert (B, Sq, Hkv, Dh) == (1, 1, _HQ, _DH)
    W = min(4096, max(256, Sk // 4))
    assert W // _LANES > max(_LEAD, _V_SPLIT)

    kt = jnp.swapaxes(A_k_cache, 2, 3)
    vt = jnp.swapaxes(A_v_cache, 2, 3)
    wq_t = _tile_groups(A_wq)
    wo_t = _tile_groups(A_wo)

    return pl.pallas_call(
        _make_kernel(D, F, Sk, W),
        out_shape=jax.ShapeDtypeStruct((B, Sq, D), A_x.dtype),
        in_specs=[pl.BlockSpec(memory_space=pl.ANY)] * 10,
        out_specs=pl.BlockSpec(memory_space=pl.ANY),
        scratch_shapes=[
            pltpu.VMEM((2, _DH, W), _BF16),
            pltpu.VMEM((2, _DH, W), _BF16),
            pltpu.VMEM(wq_t.shape, _BF16),
            pltpu.VMEM(wo_t.shape, _BF16),
            pltpu.VMEM((D, F), _BF16),
            pltpu.VMEM((F, D), _BF16),
            pltpu.VMEM((1, 1, D), _BF16),
            pltpu.VMEM((F,), _BF16),
            pltpu.VMEM((D,), _BF16),
            pltpu.VMEM((D,), _BF16),
            pltpu.VMEM((_HQ // 2, 8, 2 * _DH), _F32),
            pltpu.VMEM((8, _DH), _F32),
            pltpu.VMEM((1, 1, D), _BF16),
        ],
        compiler_params=pltpu.CompilerParams(vmem_limit_bytes=64 * 1024 * 1024),
    )(A_x, kt, vt, wq_t, wo_t, B_w1, B_b1, B_w2, B_b2, gate_w)
```

```python
import math

import jax
import jax.numpy as jnp
import jax.experimental.pallas as pl
import jax.experimental.pallas.tpu as pltpu

_F32 = jnp.float32
_BF16 = jnp.bfloat16
_LANES = 128
_SUB = 8

_HQ = 32
_DH = 192

_LEAD = 25
_ROWS_B = 128
_GROUP_TILES = 256
_GROUPS_A = 4
_MLP_GROUPS = 4
_W2_TAIL = (128, 192, 64)
_V_SPLIT = 24
_LAST_ISSUE = 8
_PART_STEPS = 40

_SEM_K, _SEM_V, _SEM_WO, _SEM_WQ, _SEM_W1, _SEM_SMALL = 0, 2, 4, 5, 6, 7
_SEM_VX, _SEM_OUT, _SEM_W2 = 11, 12, 13
_N_SEMS = _SEM_W2 + 1 + len(_W2_TAIL)


def _tile_groups(w):
    r, c = w.shape
    tiles = w.reshape(r // _SUB, _SUB, c // _LANES, _LANES).transpose(0, 2, 1, 3)
    return tiles.reshape(-1, _GROUP_TILES * _SUB, _LANES)


def _make_kernel(D, F, Sk, W):
    scale = _DH ** -0.5
    n_pairs = _HQ // 2
    pair_tiles = 2 * _DH // _LANES
    d_tiles = D // _LANES
    col0 = Sk - W
    tail_rows = F // _MLP_GROUPS
    tail0 = F - tail_rows
    nt_dims = (((1,), (1,)), ((), ()))
    group_rows = _GROUP_TILES * _SUB
    head_rows = _DH * d_tiles
    piece_rows = math.gcd(head_rows, group_rows)

    def body(x_hbm, k_hbm, v_hbm, wq_hbm, wo_hbm, w1_hbm, b1_hbm, w2_hbm, b2_hbm, gw_hbm,
             o_hbm, kbuf, vbuf, wqbuf, wobuf, w1buf, w2buf, xbuf, b1buf, b2buf, gwbuf, qbuf,
             hcolbuf, pvbuf, obuf, sems):

        def chunks(src, dst, r0, c0, n_rows, n_cols, shape, sem):
            tr, tc = shape

            def maker(r, c):
                return lambda: pltpu.make_async_copy(
                    src.at[pl.ds(r0 + r, tr), pl.ds(c0 + c, tc)],
                    dst.at[pl.ds(r0 + r, tr), pl.ds(c, tc)], sems.at[sem])

            return [maker(r, c) for r in range(0, n_rows, tr) for c in range(0, n_cols, tc)]

        def tile_steps(src, dst, g0, n_groups, sem):
            def maker(r, c):
                idx = (pl.ds(g0, n_groups), pl.ds(r, _SUB), pl.ds(c, _LANES))
                return lambda: pltpu.make_async_copy(src.at[idx], dst.at[idx], sems.at[sem])

            return [maker(r, c) for r in range(0, src.shape[1], _SUB)
                    for c in range(0, src.shape[2], _LANES)]

        def weight_phase(src, dst, sem, side):
            n, groups = len(side), src.shape[0]
            groups_b = groups - _GROUPS_A
            return (side + tile_steps(src, dst, groups_b, _GROUPS_A, sem)[n:],
                    tile_steps(src, dst, 0, groups, sem)[:n]
                    + tile_steps(src, dst, 0, groups_b, sem)[n:])

        def block(src, dst, sem, split=None):
            def slabs(sem):
                rows_a = _DH - _ROWS_B
                return (chunks(src, dst, _ROWS_B, col0, rows_a, W, (rows_a, _LANES), sem),
                        chunks(src, dst, 0, col0, _ROWS_B, W, (_ROWS_B, _LANES), sem))

            a, b = slabs(sem)
            if split is not None:
                a2, b2 = slabs(_SEM_VX)
                a, b = a[:split] + a2[split:], b[:split] + b2[split:]
            return a, b

        def k_block(h, s):
            return block(k_hbm.at[0, h], kbuf.at[s], _SEM_K + s)

        def v_block(h, s, split=None):
            return block(v_hbm.at[0, h], vbuf.at[s], _SEM_V + s, split)

        def wait_full(buf, sem):
            pltpu.make_async_copy(buf, buf, sems.at[sem]).wait()

        def issue(a, b):
            for i in range(max(len(a), len(b))):
                if i < len(b):
                    b[i]().start(priority=1)
                if i < len(a):
                    a[i]().start(priority=0)

        def tiled_matvec(lhs, w_tiles, cols):
            rows = w_tiles.shape[0] * _SUB
            return jnp.concatenate(
                [jnp.dot(lhs, w_tiles[:, c].reshape(rows, _LANES),
                         preferred_element_type=_F32) for c in cols], axis=1)

        cp_x, cp_gw, cp_b1, cp_b2 = [
            pltpu.make_async_copy(src, dst, sems.at[_SEM_SMALL + i])
            for i, (src, dst) in enumerate(
                ((x_hbm, xbuf), (gw_hbm, gwbuf), (b1_hbm, b1buf), (b2_hbm, b2buf)))
        ]
        wq_a, wq_b = weight_phase(
            wq_hbm, wqbuf, _SEM_WQ, tile_steps(w1_hbm, w1buf, 0, _MLP_GROUPS, _SEM_W1))
        wo_a, wo_b = weight_phase(
            wo_hbm, wobuf, _SEM_WO, tile_steps(w2_hbm, w2buf, 0, _MLP_GROUPS - 1, _SEM_W2))
        k0a, k0b = k_block(0, 0)
        v0a, v0b = v_block(0, 0)
        pro_a = wq_a + wo_a + k0a + v0a
        pro_b = wq_b + wo_b + k0b + v0b + k_block(1, 1)[1][:_LEAD]
        issue([], pro_b[:_LEAD])
        for cp in (cp_x, cp_gw, cp_b1, cp_b2):
            cp.start()
        pro_b = pro_b[_LEAD:]
        done = [0]

        def issue_until(n):
            issue(pro_a[done[0]:n], pro_b[done[0]:n])
            done[0] = n

        issue_until(len(wq_a) + _PART_STEPS)
        cp_x.wait()
        x = xbuf[0].astype(_F32)
        x8 = jnp.broadcast_to(x, (8, D)).astype(_BF16)
        openers = [lambda: wait_full(wqbuf, _SEM_WQ), cp_gw.wait, cp_b1.wait, cp_b2.wait]
        for part, opener in enumerate(openers):
            opener()
            wq_tiles = wqbuf[...].reshape(D // _SUB, n_pairs * pair_tiles, _SUB, _LANES)
            for p in range(part * n_pairs // len(openers), (part + 1) * n_pairs // len(openers)):
                qbuf[p] = tiled_matvec(x8, wq_tiles, range(p * pair_tiles, (p + 1) * pair_tiles))
            issue_until(done[0] + _PART_STEPS)

        wait_full(w1buf, _SEM_W1)
        gate = jax.nn.sigmoid(jnp.sum(
            x * gwbuf[...].reshape(1, D).astype(_F32), axis=-1, keepdims=True))
        hid = jnp.dot(x8, w1buf[...].reshape(D, F), preferred_element_type=_F32)
        hid = hid + b1buf[...].reshape(1, F).astype(_F32)
        hid = jax.nn.gelu(hid, approximate=True).astype(_BF16)
        tail = hid[0:1, tail0:].astype(_F32) * (1.0 - gate)
        hcolbuf[...] = jnp.broadcast_to(tail, (_LANES, tail_rows)).T
        issue_until(len(wq_a) + len(wo_a) + len(k0a))

        wait_full(wobuf, _SEM_WO)
        wait_full(w2buf.at[pl.ds(0, _MLP_GROUPS - 1)], _SEM_W2)
        mlp = b2buf[...].reshape(1, D).astype(_F32) + jnp.dot(
            hid[:, :tail0], w2buf[0:_MLP_GROUPS - 1].reshape(tail0, D),
            preferred_element_type=_F32)
        issue_until(len(pro_a))

        def scores(q, s):
            wait_full(kbuf.at[s], _SEM_K + s)
            sc = jnp.dot(q, kbuf[s], preferred_element_type=_F32) * scale
            e = jnp.exp(sc - jnp.max(sc, axis=-1, keepdims=True))
            return e.astype(_BF16), jnp.sum(e, axis=-1, keepdims=True)

        def out_proj(o, l, h):
            pieces = []
            for r in range(0, head_rows, piece_rows):
                r = h * head_rows + r
                if isinstance(r, int):
                    g, off = divmod(r, group_rows)
                else:
                    g = jax.lax.div(r, group_rows)
                    off = pl.multiple_of(jax.lax.rem(r, group_rows), piece_rows)
                pieces.append(wobuf[g, pl.ds(off, piece_rows), :])
            wo_h = jnp.concatenate(pieces, axis=0).reshape(_DH // _SUB, d_tiles, _SUB, _LANES)
            return tiled_matvec((o / l).astype(_BF16), wo_h, range(d_tiles))

        def project(e, l, s, h):
            wait_full(vbuf.at[s], _SEM_V + s)
            o = jax.lax.dot_general(e, vbuf[s], nt_dims, preferred_element_type=_F32)
            return out_proj(o, l, h)

        def pair_step(p, acc):
            h = 2 * p
            k1a, k1b = k_block(h + 1, 1)
            v1a, v1b = v_block(h + 1, 1)
            k2a, k2b = k_block(h + 2, 0)
            v2a, v2b = v_block(h + 2, 0)
            issue(k1a, k1b[_LEAD:] + v1b[:_LEAD])
            q2 = qbuf[p].astype(_BF16)
            e, l = scores(q2[:, :_DH], 0)
            issue(v1a, v1b[_LEAD:] + k2b[:_LEAD])
            acc = acc + project(e, l, 0, h)
            issue(k2a, k2b[_LEAD:] + v2b[:_LEAD])
            e, l = scores(q2[:, _DH:], 1)
            issue(v2a, v2b[_LEAD:] + k_block(h + 3, 1)[1][:_LEAD])
            return acc + project(e, l, 1, h + 1)

        acc = jax.lax.fori_loop(0, n_pairs - 1, pair_step, jnp.zeros((8, D), _F32))

        h = _HQ - 2
        k1a, k1b = k_block(h + 1, 1)
        v1a, v1b = v_block(h + 1, 1, _V_SPLIT)
        w2_tail_hbm, w2_tail = w2_hbm.at[_MLP_GROUPS - 1], w2buf.at[_MLP_GROUPS - 1]
        b_end, r0 = v1b[_LEAD:], 0
        for i, rows in enumerate(_W2_TAIL):
            b_end += chunks(w2_tail_hbm, w2_tail, r0, 0, rows, D, (16, D), _SEM_W2 + 1 + i)
            r0 += rows
        issue(k1a, k1b[_LEAD:] + v1b[:_LEAD])
        q2 = qbuf[n_pairs - 1].astype(_BF16)
        e, l = scores(q2[:, :_DH], 0)
        issue(v1a[:_LAST_ISSUE], b_end[:_LAST_ISSUE])
        acc = acc + project(e, l, 0, h)
        issue(v1a[_LAST_ISSUE:], b_end[_LAST_ISSUE:])
        e, l = scores(q2[:, _DH:], 1)
        cs = _V_SPLIT * _LANES
        wait_full(vbuf.at[1, :, pl.ds(0, cs)], _SEM_V + 1)
        pvbuf[...] = jax.lax.dot_general(e[:, :cs], vbuf[1, :, :cs], nt_dims,
                                         preferred_element_type=_F32)
        wait_full(vbuf.at[1, :, pl.ds(cs, W - cs)], _SEM_VX)
        o = pvbuf[...] + jax.lax.dot_general(e[:, cs:], vbuf[1, :, cs:], nt_dims,
                                             preferred_element_type=_F32)
        att = acc + out_proj(o, l, h + 1)

        base = gate * att + (1.0 - gate) * mlp
        row = jax.lax.broadcasted_iota(jnp.int32, (8, D), 0)
        part = jnp.where(row == 0, base, 0.0)
        r0 = 0
        for i, rows in enumerate(_W2_TAIL):
            wait_full(w2_tail.at[pl.ds(r0, rows)], _SEM_W2 + 1 + i)
            hcol = hcolbuf[r0:r0 + rows, :]
            sums = []
            for c in range(d_tiles):
                w = w2_tail[r0:r0 + rows, c * _LANES:(c + 1) * _LANES].astype(_F32)
                sums.append(jnp.sum((w * hcol).reshape(rows // 8, 8, _LANES), axis=0))
            part = part + jnp.concatenate(sums, axis=1)
            r0 += rows
        obuf[0] = jnp.sum(part, axis=0, keepdims=True).astype(obuf.dtype)
        out_copy = pltpu.make_async_copy(obuf, o_hbm, sems.at[_SEM_OUT])
        out_copy.start()
        out_copy.wait()

    def kernel(*refs):
        pl.run_scoped(lambda sems: body(*refs, sems), pltpu.SemaphoreType.DMA((_N_SEMS,)))

    return kernel


@jax.jit
def pallas_gated_mix__sliding_block_cached__dense_activation_gelu__decode_kernel(
    A_x: jax.Array,
    A_k_cache: jax.Array,
    A_v_cache: jax.Array,
    A_wq: jax.Array,
    A_wo: jax.Array,
    B_x: jax.Array,
    B_w1: jax.Array,
    B_b1: jax.Array,
    B_w2: jax.Array,
    B_b2: jax.Array,
    gate_w: jax.Array,
):
    del B_x
    B, Sq, D = A_x.shape
    _, Hkv, Sk, Dh = A_k_cache.shape
    F = B_w1.shape[1]
    assert (B, Sq, Hkv, Dh) == (1, 1, _HQ, _DH)
    assert sum(_W2_TAIL) * _MLP_GROUPS == F
    W = min(4096, max(256, Sk // 4))
    assert W // _LANES > max(_LEAD, _V_SPLIT)

    kt = jnp.swapaxes(A_k_cache, 2, 3)
    vt = jnp.swapaxes(A_v_cache, 2, 3)
    wq_t = _tile_groups(A_wq)
    wo_t = _tile_groups(A_wo)
    w1_g = B_w1.reshape(_MLP_GROUPS, D // _MLP_GROUPS, F)
    w2_g = B_w2.reshape(_MLP_GROUPS, F // _MLP_GROUPS, D)

    return pl.pallas_call(
        _make_kernel(D, F, Sk, W),
        out_shape=jax.ShapeDtypeStruct((B, Sq, D), A_x.dtype),
        in_specs=[pl.BlockSpec(memory_space=pl.ANY)] * 10,
        out_specs=pl.BlockSpec(memory_space=pl.ANY),
        scratch_shapes=[
            pltpu.VMEM((2, _DH, W), _BF16),
            pltpu.VMEM((2, _DH, W), _BF16),
            pltpu.VMEM(wq_t.shape, _BF16),
            pltpu.VMEM(wo_t.shape, _BF16),
            pltpu.VMEM(w1_g.shape, _BF16),
            pltpu.VMEM(w2_g.shape, _BF16),
            pltpu.VMEM((1, 1, D), _BF16),
            pltpu.VMEM((F,), _BF16),
            pltpu.VMEM((D,), _BF16),
            pltpu.VMEM((D,), _BF16),
            pltpu.VMEM((_HQ // 2, 8, 2 * _DH), _F32),
            pltpu.VMEM((F // _MLP_GROUPS, _LANES), _F32),
            pltpu.VMEM((8, _DH), _F32),
            pltpu.VMEM((1, 1, D), _BF16),
        ],
        compiler_params=pltpu.CompilerParams(vmem_limit_bytes=64 * 1024 * 1024),
    )(A_x, kt, vt, wq_t, wo_t, w1_g, B_b1, w2_g, B_b2, gate_w)
```

```python
import math

import jax
import jax.numpy as jnp
import jax.experimental.pallas as pl
import jax.experimental.pallas.tpu as pltpu

_F32 = jnp.float32
_BF16 = jnp.bfloat16
_LANES = 128
_SUB = 8

_HQ = 32
_DH = 192

_LEAD = 25
_ROWS_B = 128
_GROUP_TILES = 256
_GROUPS_A = 4
_MLP_GROUPS = 4
_W2_TAIL = (256, 96, 32)
_V_SPLITS = (18, 27)
_LAST_ISSUE = 8
_PART_STEPS = 40

_SEM_K, _SEM_V, _SEM_WO, _SEM_WQ, _SEM_W1, _SEM_SMALL = 0, 2, 4, 5, 6, 7
_SEM_OUT, _SEM_W2 = 11, 12
_SEM_VX = _SEM_W2 + 1 + len(_W2_TAIL)
_N_SEMS = _SEM_VX + len(_V_SPLITS)


def _tile_groups(w):
    r, c = w.shape
    tiles = w.reshape(r // _SUB, _SUB, c // _LANES, _LANES).transpose(0, 2, 1, 3)
    return tiles.reshape(-1, _GROUP_TILES * _SUB, _LANES)


def _make_kernel(D, F, Sk, W):
    scale = _DH ** -0.5
    n_pairs = _HQ // 2
    pair_tiles = 2 * _DH // _LANES
    d_tiles = D // _LANES
    col0 = Sk - W
    tail_rows = F // _MLP_GROUPS
    tail0 = F - tail_rows
    nt_dims = (((1,), (1,)), ((), ()))
    group_rows = _GROUP_TILES * _SUB
    head_rows = _DH * d_tiles
    piece_rows = math.gcd(head_rows, group_rows)

    def body(x_hbm, k_hbm, v_hbm, wq_hbm, wo_hbm, w1_hbm, b1_hbm, w2_hbm, b2_hbm, gw_hbm,
             o_hbm, kbuf, vbuf, wqbuf, wobuf, w1buf, w2buf, xbuf, b1buf, b2buf, gwbuf, qbuf,
             hcolbuf, pvbuf, obuf, sems):

        def chunks(src, dst, r0, c0, n_rows, n_cols, shape, sem):
            tr, tc = shape

            def maker(r, c):
                return lambda: pltpu.make_async_copy(
                    src.at[pl.ds(r0 + r, tr), pl.ds(c0 + c, tc)],
                    dst.at[pl.ds(r0 + r, tr), pl.ds(c, tc)], sems.at[sem])

            return [maker(r, c) for r in range(0, n_rows, tr) for c in range(0, n_cols, tc)]

        def tile_steps(src, dst, g0, n_groups, sem):
            def maker(r, c):
                idx = (pl.ds(g0, n_groups), pl.ds(r, _SUB), pl.ds(c, _LANES))
                return lambda: pltpu.make_async_copy(src.at[idx], dst.at[idx], sems.at[sem])

            return [maker(r, c) for r in range(0, src.shape[1], _SUB)
                    for c in range(0, src.shape[2], _LANES)]

        def weight_phase(src, dst, sem, side):
            n, groups = len(side), src.shape[0]
            assert n <= _GROUP_TILES
            groups_b = groups - _GROUPS_A
            return (side + tile_steps(src, dst, groups_b, _GROUPS_A, sem)[n:],
                    tile_steps(src, dst, 0, groups, sem)[:n]
                    + tile_steps(src, dst, 0, groups_b, sem)[n:])

        def block(src, dst, sem, splits=()):
            def slabs(sem):
                rows_a = _DH - _ROWS_B
                return (chunks(src, dst, _ROWS_B, col0, rows_a, W, (rows_a, _LANES), sem),
                        chunks(src, dst, 0, col0, _ROWS_B, W, (_ROWS_B, _LANES), sem))

            a, b = slabs(sem)
            for i, cut in enumerate(splits):
                a2, b2 = slabs(_SEM_VX + i)
                a, b = a[:cut] + a2[cut:], b[:cut] + b2[cut:]
            return a, b

        def k_block(h, s):
            return block(k_hbm.at[0, h], kbuf.at[s], _SEM_K + s)

        def v_block(h, s, splits=()):
            return block(v_hbm.at[0, h], vbuf.at[s], _SEM_V + s, splits)

        def wait_full(buf, sem):
            pltpu.make_async_copy(buf, buf, sems.at[sem]).wait()

        def issue(a, b):
            for i in range(max(len(a), len(b))):
                if i < len(b):
                    b[i]().start(priority=1)
                if i < len(a):
                    a[i]().start(priority=0)

        def tiled_matvec(lhs, w_tiles, cols):
            rows = w_tiles.shape[0] * _SUB
            return jnp.concatenate(
                [jnp.dot(lhs, w_tiles[:, c].reshape(rows, _LANES),
                         preferred_element_type=_F32) for c in cols], axis=1)

        cp_x, cp_gw, cp_b1, cp_b2 = [
            pltpu.make_async_copy(src, dst, sems.at[_SEM_SMALL + i])
            for i, (src, dst) in enumerate(
                ((x_hbm, xbuf), (gw_hbm, gwbuf), (b1_hbm, b1buf), (b2_hbm, b2buf)))
        ]
        wq_a, wq_b = weight_phase(
            wq_hbm, wqbuf, _SEM_WQ, tile_steps(w1_hbm, w1buf, 0, _MLP_GROUPS, _SEM_W1))
        wo_a, wo_b = weight_phase(
            wo_hbm, wobuf, _SEM_WO, tile_steps(w2_hbm, w2buf, 0, _MLP_GROUPS - 1, _SEM_W2))
        k0a, k0b = k_block(0, 0)
        v0a, v0b = v_block(0, 0)
        pro_a = wq_a + wo_a + k0a + v0a
        pro_b = wq_b + wo_b + k0b + v0b + k_block(1, 1)[1][:_LEAD]
        issue([], pro_b[:_LEAD])
        for cp in (cp_x, cp_gw, cp_b1, cp_b2):
            cp.start()
        pro_b = pro_b[_LEAD:]
        done = [0]

        def issue_until(n):
            assert done[0] <= n <= len(pro_a) == len(pro_b)
            issue(pro_a[done[0]:n], pro_b[done[0]:n])
            done[0] = n

        issue_until(len(wq_a) + _PART_STEPS)
        cp_x.wait()
        x = xbuf[0].astype(_F32)
        x8 = jnp.broadcast_to(x, (8, D)).astype(_BF16)
        openers = [lambda: wait_full(wqbuf, _SEM_WQ), cp_gw.wait, cp_b1.wait, cp_b2.wait]
        for part, opener in enumerate(openers):
            opener()
            wq_tiles = wqbuf[...].reshape(D // _SUB, n_pairs * pair_tiles, _SUB, _LANES)
            for p in range(part * n_pairs // len(openers), (part + 1) * n_pairs // len(openers)):
                qbuf[p] = tiled_matvec(x8, wq_tiles, range(p * pair_tiles, (p + 1) * pair_tiles))
            issue_until(done[0] + _PART_STEPS)

        wait_full(w1buf, _SEM_W1)
        gate = jax.nn.sigmoid(jnp.sum(
            x * gwbuf[...].reshape(1, D).astype(_F32), axis=-1, keepdims=True))
        hid = jnp.dot(x8, w1buf[...].reshape(D, F), preferred_element_type=_F32)
        hid = hid + b1buf[...].reshape(1, F).astype(_F32)
        hid = jax.nn.gelu(hid, approximate=True).astype(_BF16)
        tail = hid[0:1, tail0:].astype(_F32) * (1.0 - gate)
        hcolbuf[...] = jnp.broadcast_to(tail, (_LANES, tail_rows)).T
        issue_until(len(wq_a) + len(wo_a) + len(k0a))

        wait_full(wobuf, _SEM_WO)
        wait_full(w2buf.at[pl.ds(0, _MLP_GROUPS - 1)], _SEM_W2)
        mlp = b2buf[...].reshape(1, D).astype(_F32) + jnp.dot(
            hid[:, :tail0], w2buf[0:_MLP_GROUPS - 1].reshape(tail0, D),
            preferred_element_type=_F32)
        issue_until(len(pro_a))

        def scores(q, s):
            wait_full(kbuf.at[s], _SEM_K + s)
            sc = jnp.dot(q, kbuf[s], preferred_element_type=_F32) * scale
            e = jnp.exp(sc - jnp.max(sc, axis=-1, keepdims=True))
            return e.astype(_BF16), jnp.sum(e, axis=-1, keepdims=True)

        def out_proj(o, l, h):
            pieces = []
            for r in range(0, head_rows, piece_rows):
                r = h * head_rows + r
                if isinstance(r, int):
                    g, off = divmod(r, group_rows)
                else:
                    g = jax.lax.div(r, group_rows)
                    off = pl.multiple_of(jax.lax.rem(r, group_rows), piece_rows)
                pieces.append(wobuf[g, pl.ds(off, piece_rows), :])
            wo_h = jnp.concatenate(pieces, axis=0).reshape(_DH // _SUB, d_tiles, _SUB, _LANES)
            return tiled_matvec((o / l).astype(_BF16), wo_h, range(d_tiles))

        def project(e, l, s, h):
            wait_full(vbuf.at[s], _SEM_V + s)
            o = jax.lax.dot_general(e, vbuf[s], nt_dims, preferred_element_type=_F32)
            return out_proj(o, l, h)

        def pair_step(p, acc):
            h = 2 * p
            k1a, k1b = k_block(h + 1, 1)
            v1a, v1b = v_block(h + 1, 1)
            k2a, k2b = k_block(h + 2, 0)
            v2a, v2b = v_block(h + 2, 0)
            issue(k1a, k1b[_LEAD:] + v1b[:_LEAD])
            q2 = qbuf[p].astype(_BF16)
            e, l = scores(q2[:, :_DH], 0)
            issue(v1a, v1b[_LEAD:] + k2b[:_LEAD])
            acc = acc + project(e, l, 0, h)
            issue(k2a, k2b[_LEAD:] + v2b[:_LEAD])
            e, l = scores(q2[:, _DH:], 1)
            issue(v2a, v2b[_LEAD:] + k_block(h + 3, 1)[1][:_LEAD])
            return acc + project(e, l, 1, h + 1)

        acc = jax.lax.fori_loop(0, n_pairs - 1, pair_step, jnp.zeros((8, D), _F32))

        h = _HQ - 2
        k1a, k1b = k_block(h + 1, 1)
        v1a, v1b = v_block(h + 1, 1, _V_SPLITS)
        w2_tail_hbm, w2_tail = w2_hbm.at[_MLP_GROUPS - 1], w2buf.at[_MLP_GROUPS - 1]
        b_end, r0 = v1b[_LEAD:], 0
        for i, rows in enumerate(_W2_TAIL):
            b_end += chunks(w2_tail_hbm, w2_tail, r0, 0, rows, D, (16, D), _SEM_W2 + 1 + i)
            r0 += rows
        issue(k1a, k1b[_LEAD:] + v1b[:_LEAD])
        q2 = qbuf[n_pairs - 1].astype(_BF16)
        e, l = scores(q2[:, :_DH], 0)
        issue(v1a[:_LAST_ISSUE], b_end[:_LAST_ISSUE])
        acc = acc + project(e, l, 0, h)
        issue(v1a[_LAST_ISSUE:], b_end[_LAST_ISSUE:])
        e, l = scores(q2[:, _DH:], 1)
        edges = [0] + [cut * _LANES for cut in _V_SPLITS] + [W]
        for i, (lo, hi) in enumerate(zip(edges[:-1], edges[1:])):
            wait_full(vbuf.at[1, :, pl.ds(lo, hi - lo)], _SEM_VX + i - 1 if i else _SEM_V + 1)
            o = jax.lax.dot_general(e[:, lo:hi], vbuf[1, :, lo:hi], nt_dims,
                                    preferred_element_type=_F32)
            if i > 0:
                o = pvbuf[...] + o
            if hi < W:
                pvbuf[...] = o
        att = acc + out_proj(o, l, h + 1)

        base = gate * att + (1.0 - gate) * mlp
        row = jax.lax.broadcasted_iota(jnp.int32, (8, D), 0)
        part = jnp.where(row == 0, base, 0.0)
        r0 = 0
        for i, rows in enumerate(_W2_TAIL):
            wait_full(w2_tail.at[pl.ds(r0, rows)], _SEM_W2 + 1 + i)
            hcol = hcolbuf[r0:r0 + rows, :]
            sums = []
            for c in range(d_tiles):
                w = w2_tail[r0:r0 + rows, c * _LANES:(c + 1) * _LANES].astype(_F32)
                sums.append(jnp.sum((w * hcol).reshape(rows // 8, 8, _LANES), axis=0))
            part = part + jnp.concatenate(sums, axis=1)
            r0 += rows
        obuf[0] = jnp.sum(part, axis=0, keepdims=True).astype(obuf.dtype)
        out_copy = pltpu.make_async_copy(obuf, o_hbm, sems.at[_SEM_OUT])
        out_copy.start()
        out_copy.wait()

    def kernel(*refs):
        pl.run_scoped(lambda sems: body(*refs, sems), pltpu.SemaphoreType.DMA((_N_SEMS,)))

    return kernel


@jax.jit
def pallas_gated_mix__sliding_block_cached__dense_activation_gelu__decode_kernel(
    A_x: jax.Array,
    A_k_cache: jax.Array,
    A_v_cache: jax.Array,
    A_wq: jax.Array,
    A_wo: jax.Array,
    B_x: jax.Array,
    B_w1: jax.Array,
    B_b1: jax.Array,
    B_w2: jax.Array,
    B_b2: jax.Array,
    gate_w: jax.Array,
):
    del B_x
    B, Sq, D = A_x.shape
    _, Hkv, Sk, Dh = A_k_cache.shape
    F = B_w1.shape[1]
    assert (B, Sq, Hkv, Dh) == (1, 1, _HQ, _DH)
    assert sum(_W2_TAIL) * _MLP_GROUPS == F
    W = min(4096, max(256, Sk // 4))
    assert W // _LANES > max(_LEAD, *_V_SPLITS)

    kt = jnp.swapaxes(A_k_cache, 2, 3)
    vt = jnp.swapaxes(A_v_cache, 2, 3)
    wq_t = _tile_groups(A_wq)
    wo_t = _tile_groups(A_wo)
    w1_g = B_w1.reshape(_MLP_GROUPS, D // _MLP_GROUPS, F)
    w2_g = B_w2.reshape(_MLP_GROUPS, F // _MLP_GROUPS, D)

    return pl.pallas_call(
        _make_kernel(D, F, Sk, W),
        out_shape=jax.ShapeDtypeStruct((B, Sq, D), A_x.dtype),
        in_specs=[pl.BlockSpec(memory_space=pl.ANY)] * 10,
        out_specs=pl.BlockSpec(memory_space=pl.ANY),
        scratch_shapes=[
            pltpu.VMEM((2, _DH, W), _BF16),
            pltpu.VMEM((2, _DH, W), _BF16),
            pltpu.VMEM(wq_t.shape, _BF16),
            pltpu.VMEM(wo_t.shape, _BF16),
            pltpu.VMEM(w1_g.shape, _BF16),
            pltpu.VMEM(w2_g.shape, _BF16),
            pltpu.VMEM((1, 1, D), _BF16),
            pltpu.VMEM((F,), _BF16),
            pltpu.VMEM((D,), _BF16),
            pltpu.VMEM((D,), _BF16),
            pltpu.VMEM((_HQ // 2, 8, 2 * _DH), _F32),
            pltpu.VMEM((F // _MLP_GROUPS, _LANES), _F32),
            pltpu.VMEM((8, _DH), _F32),
            pltpu.VMEM((1, 1, D), _BF16),
        ],
        compiler_params=pltpu.CompilerParams(vmem_limit_bytes=64 * 1024 * 1024),
    )(A_x, kt, vt, wq_t, wo_t, w1_g, B_b1, w2_g, B_b2, gate_w)
```
